```python
import jax
import jax.numpy as jnp

def _softmax(x, axis=-1):
    return jax.nn.softmax(x, axis=axis)

def _gelu(x):
    return jax.nn.gelu(x, approximate=True)

def _silu(x):
    return jax.nn.silu(x)

def _sigmoid(x):
    return jax.nn.sigmoid(x)

def _layernorm(x, axis=-1, eps=1e-05):
    m = jnp.mean(x, axis=axis, keepdims=True)
    v = jnp.var(x, axis=axis, keepdims=True)
    return (x - m) / jnp.sqrt(v + eps)

def _scatter_add(tgt, idx, src, axis=0):
    return tgt.at[idx].add(src)

def _segment_sum(src, seg, n):
    return jax.ops.segment_sum(src, seg, n)

class _Rng:

    def __init__(self, key):
        self._k = key

    def _next(self):
        self._k, sub = jax.random.split(self._k)
        return sub

    def normal(self, shape):
        return jax.random.normal(self._next(), shape, dtype=jnp.bfloat16)

    def randint(self, lo, hi, shape):
        return jax.random.randint(self._next(), shape, lo, hi, dtype=jnp.int32)

    def uniform(self, shape, lo=0.0, hi=1.0):
        return jax.random.uniform(self._next(), shape, jnp.bfloat16, lo, hi)

    def permutation(self, n):
        return jax.random.permutation(self._next(), n)
kernel_name = 'adaLN_cond__sliding_block_cached__glu_gated_bilinear__decode'

def setup_inputs():
    _rng = _Rng(jax.random.key(int.from_bytes(__import__("os").urandom(4), "little")))
    _w = lambda a: (lambda t: t.astype(jnp.bfloat16) if jnp.issubdtype(t.dtype, jnp.floating) else t)(jnp.asarray(a))

    def _A_setup():
        B, Sq, D = (1, 1, 640)
        Hq, Hkv, Sk, Dh = (32, 32, 32768, 192)
        assert Hq % Hkv == 0, (Hq, Hkv)
        return {'x': _w((lambda *s: _rng.normal(s) * 0.05)(B, Sq, D)), 'k_cache': _w((lambda *s: _rng.normal(s) * 0.05)(B, Hkv, Sk, Dh)), 'v_cache': _w((lambda *s: _rng.normal(s) * 0.05)(B, Hkv, Sk, Dh)), 'wq': _w((lambda *s: _rng.normal(s) * 0.05)(D, Hq * Dh) * D ** (-0.5)), 'wo': _w((lambda *s: _rng.normal(s) * 0.05)(Hq * Dh, D) * (Hq * Dh) ** (-0.5))}
    _A_in = _A_setup()

    def _B_setup():
        B, S, D, F = (1, 1, 640, 1536)
        return {'x': _w((lambda *s: _rng.normal(s) * 0.05)(B, S, D)), 'w_gate': _w((lambda *s: _rng.normal(s) * 0.05)(D, F) * D ** (-0.5)), 'w_up': _w((lambda *s: _rng.normal(s) * 0.05)(D, F) * D ** (-0.5)), 'w_down': _w((lambda *s: _rng.normal(s) * 0.05)(F, D) * F ** (-0.5))}
    _B_in = _B_setup()
    return {'A_x': _A_in['x'], 'A_k_cache': _A_in['k_cache'], 'A_v_cache': _A_in['v_cache'], 'A_wq': _A_in['wq'], 'A_wo': _A_in['wo'], 'B_x': _B_in['x'], 'B_w_gate': _B_in['w_gate'], 'B_w_up': _B_in['w_up'], 'B_w_down': _B_in['w_down'], 'c': _w((lambda *s: _rng.normal(s) * 0.05)(1, 640)), 'w_mod': _w((lambda *s: _rng.normal(s) * 0.05)(640, 6 * 640) * 640 ** (-0.5))}

def reference(A_x, A_k_cache, A_v_cache, A_wq, A_wo, B_x, B_w_gate, B_w_up, B_w_down, c, w_mod):

    def _A_ref(x, k_cache, v_cache, wq, wo):
        B, Sq, D = x.shape
        Hq, Dh = (32, 192)
        Hkv, Sk = (k_cache.shape[1], k_cache.shape[2])
        W = min(4096, max(256, Sk // 4))
        rep = Hq // Hkv
        q = (lambda x, *d: x.transpose(*d))((x @ wq).reshape(B, Sq, Hq, Dh), 0, 2, 1, 3)
        k = jnp.repeat(k_cache[:, :, Sk - W:, :], rep, axis=1)
        v = jnp.repeat(v_cache[:, :, Sk - W:, :], rep, axis=1)
        scores = jnp.einsum('bhqd,bhkd->bhqk', q, k) * Dh ** (-0.5)
        p = _softmax(scores, axis=-1)
        o = jnp.einsum('bhqk,bhkd->bhqd', p, v)
        return (lambda x, *d: x.transpose(*d))(o, 0, 2, 1, 3).reshape(B, Sq, Hq * Dh) @ wo

    def _B_ref(x, w_gate, w_up, w_down):
        g = jnp.einsum('bsd,df->bsf', x, w_gate)
        u = jnp.einsum('bsd,df->bsf', x, w_up)
        h = g * u
        return jnp.einsum('bsf,fd->bsd', h, w_down)
    x = A_x
    mod = (_silu(c) @ w_mod).reshape(c.shape[0], 6, 1, -1)
    sa, ca, ga, sb, cb, gb = (mod[:, 0].copy(), mod[:, 1].copy(), mod[:, 2].copy(), mod[:, 3].copy(), mod[:, 4].copy(), mod[:, 5].copy())
    h = _layernorm(x, axis=-1) * (1 + ca) + sa
    x = x + ga * _A_ref(h, A_k_cache, A_v_cache, A_wq, A_wo)
    h = _layernorm(x, axis=-1) * (1 + cb) + sb
    x = x + gb * _B_ref(h, B_w_gate, B_w_up, B_w_down)
    return x
```

```python
import functools
import jax
import jax.numpy as jnp
from jax import lax
import jax.experimental.pallas as pl
import jax.experimental.pallas.tpu as pltpu

F32 = jnp.float32
BF16 = jnp.bfloat16


def _layernorm(x, eps=1e-5):
    m = jnp.mean(x, axis=-1, keepdims=True)
    xc = x - m
    v = jnp.mean(xc * xc, axis=-1, keepdims=True)
    return xc * lax.rsqrt(v + eps)


def build(G=2, R=4, WO_CH=4, WD_CH=2, debug=False):
    D, H, Dh, F = 640, 32, 192, 1536
    NG = H // G
    GD = G * Dh
    M = 8
    scale = Dh ** -0.5

    def make(Sk, W):
        def kernel(x_hbm, c_hbm, k_hbm, v_hbm, wq_hbm, wo_hbm, wg_hbm, wu_hbm, wd_hbm, wm_hbm,
                   o_ref,
                   x_v, c_v, wm_v, wq_v, wo_v, wg_v, wu_v, wd_v, kbuf, vbuf, q_s, o_s,
                   sem_misc, sem_k, sem_v, sem_wo, sem_wd, sem_gb):
            def cp_k(g, slot):
                return pltpu.make_async_copy(
                    k_hbm.at[pl.ds(g * GD, GD), pl.ds(Sk - W, W)], kbuf.at[slot], sem_k.at[slot])

            def cp_v(g, slot):
                return pltpu.make_async_copy(
                    v_hbm.at[pl.ds(g * GD, GD), pl.ds(Sk - W, W)], vbuf.at[slot], sem_v.at[slot])

            cp_c = pltpu.make_async_copy(c_hbm, c_v, sem_misc.at[0])
            cp_x = pltpu.make_async_copy(x_hbm, x_v, sem_misc.at[1])
            cp_wm = pltpu.make_async_copy(wm_hbm.at[:, pl.ds(0, 5 * D)], wm_v.at[:, pl.ds(0, 5 * D)], sem_misc.at[2])
            cp_wq = pltpu.make_async_copy(wq_hbm, wq_v, sem_misc.at[3])
            cp_wg = pltpu.make_async_copy(wg_hbm, wg_v, sem_misc.at[4])
            cp_wu = pltpu.make_async_copy(wu_hbm, wu_v, sem_misc.at[5])
            wo_rows = H * Dh // WO_CH
            cp_wo = [pltpu.make_async_copy(wo_hbm.at[pl.ds(i * wo_rows, wo_rows), :],
                                           wo_v.at[pl.ds(i * wo_rows, wo_rows), :], sem_wo.at[i])
                     for i in range(WO_CH)]
            wd_rows = F // WD_CH
            cp_wd = [pltpu.make_async_copy(wd_hbm.at[pl.ds(i * wd_rows, wd_rows), :],
                                           wd_v.at[pl.ds(i * wd_rows, wd_rows), :], sem_wd.at[i])
                     for i in range(WD_CH)]
            gb_splits = [(0, 512), (512, 128)]
            cp_gb = [pltpu.make_async_copy(wm_hbm.at[pl.ds(r0, n), pl.ds(5 * D, D)],
                                           wm_v.at[pl.ds(r0, n), pl.ds(5 * D, D)], sem_gb.at[i])
                     for i, (r0, n) in enumerate(gb_splits)]

            def start_tail():
                for cp in cp_wo:
                    cp.start()
                cp_wg.start()
                cp_wu.start()
                for cp in cp_wd:
                    cp.start()
                for cp in cp_gb:
                    cp.start()

            cp_c.start()
            cp_x.start()
            cp_wm.start()
            cp_wq.start()
            for g in range(R):
                cp_k(g, g).start()
                cp_v(g, g).start()
            if R >= NG:
                start_tail()

            cp_c.wait()
            cp_x.wait()
            c = c_v[...].astype(F32)
            sc = c * (1.0 / (1.0 + jnp.exp(-c)))
            sc8 = jnp.broadcast_to(sc, (M, D)).astype(BF16)
            x = x_v[...].reshape(1, D).astype(F32)
            x8 = jnp.broadcast_to(x, (M, D))
            ln_x = _layernorm(x8)
            cp_wm.wait()
            mod = jnp.dot(sc8, wm_v[:, 0:5 * D], preferred_element_type=F32)
            sa = mod[:, 0 * D:1 * D]
            ca = mod[:, 1 * D:2 * D]
            ga = mod[:, 2 * D:3 * D]
            sb = mod[:, 3 * D:4 * D]
            cb = mod[:, 4 * D:5 * D]
            h = (ln_x * (1.0 + ca) + sa).astype(BF16)

            row = lax.broadcasted_iota(jnp.int32, (M, GD), 0)
            col = lax.broadcasted_iota(jnp.int32, (M, GD), 1)
            diag = (col >= row * Dh) & (col < (row + 1) * Dh)
            cp_wq.wait()
            for g in range(NG):
                qg = jnp.dot(h, wq_v[:, g * GD:(g + 1) * GD], preferred_element_type=F32)
                q_s[g] = jnp.where(diag, qg, 0.0).astype(BF16)

            def body(g, carry):
                slot = g % R
                cp_k(g, slot).wait()
                s = jnp.dot(q_s[g], kbuf[slot], preferred_element_type=F32) * scale

                @pl.when(g + R < NG)
                def _():
                    cp_k(g + R, slot).start()

                m = jnp.max(s, axis=-1, keepdims=True)
                p = jnp.exp(s - m)
                l = jnp.sum(p, axis=-1, keepdims=True)
                cp_v(g, slot).wait()
                o = lax.dot_general(p.astype(BF16), vbuf[slot], (((1,), (1,)), ((), ())),
                                    preferred_element_type=F32)
                o_s[g] = jnp.where(diag, o / l, 0.0).astype(BF16)

                @pl.when(g + R < NG)
                def _():
                    cp_v(g + R, slot).start()

                if R < NG:
                    @pl.when(g + R == NG - 1)
                    def _():
                        start_tail()
                return carry

            lax.fori_loop(0, NG, body, 0)

            gpc = NG // WO_CH
            acc = jnp.zeros((M, D), F32)
            for i in range(WO_CH):
                cp_wo[i].wait()
                for g in range(i * gpc, (i + 1) * gpc):
                    acc = acc + jnp.dot(o_s[g], wo_v[g * GD:(g + 1) * GD, :], preferred_element_type=F32)
            attn = jnp.sum(acc, axis=0, keepdims=True)
            x1 = x8 + ga * attn
            h2 = (_layernorm(x1) * (1.0 + cb) + sb).astype(BF16)

            cp_wg.wait()
            gg = jnp.dot(h2, wg_v[...], preferred_element_type=F32)
            cp_wu.wait()
            uu = jnp.dot(h2, wu_v[...], preferred_element_type=F32)
            hh = (gg * uu).astype(BF16)
            ffn = jnp.zeros((M, D), F32)
            for i in range(WD_CH):
                cp_wd[i].wait()
                ffn = ffn + jnp.dot(hh[:, i * wd_rows:(i + 1) * wd_rows], wd_v[i * wd_rows:(i + 1) * wd_rows, :],
                                    preferred_element_type=F32)
            gb = jnp.zeros((M, D), F32)
            for i, (r0, n) in enumerate(gb_splits):
                cp_gb[i].wait()
                gb = gb + jnp.dot(sc8[:, r0:r0 + n], wm_v[r0:r0 + n, 5 * D:6 * D], preferred_element_type=F32)
            out = x1 + gb * ffn
            if debug:
                o_ref[0] = out[0:1]
                o_ref[1] = attn
                o_ref[2] = ffn[0:1]
            else:
                o_ref[...] = out[0:1].reshape(1, 1, D).astype(o_ref.dtype)
        return kernel

    @jax.jit
    def fn(A_x, A_k_cache, A_v_cache, A_wq, A_wo, B_x, B_w_gate, B_w_up, B_w_down, c, w_mod):
        Sk = A_k_cache.shape[2]
        W = min(4096, max(256, Sk // 4))
        kt = jnp.swapaxes(A_k_cache, 2, 3).reshape(H * Dh, Sk)
        vt = jnp.swapaxes(A_v_cache, 2, 3).reshape(H * Dh, Sk)
        any_spec = pl.BlockSpec(memory_space=pl.ANY)
        out_shape = jax.ShapeDtypeStruct((3, 1, D), F32) if debug else jax.ShapeDtypeStruct((1, 1, D), A_x.dtype)
        return pl.pallas_call(
            make(Sk, W),
            out_shape=out_shape,
            in_specs=[any_spec] * 10,
            scratch_shapes=[
                pltpu.VMEM((1, 1, D), BF16),
                pltpu.VMEM((1, D), BF16),
                pltpu.VMEM((D, 6 * D), BF16),
                pltpu.VMEM((D, H * Dh), BF16),
                pltpu.VMEM((H * Dh, D), BF16),
                pltpu.VMEM((D, F), BF16),
                pltpu.VMEM((D, F), BF16),
                pltpu.VMEM((F, D), BF16),
                pltpu.VMEM((R, GD, W), BF16),
                pltpu.VMEM((R, GD, W), BF16),
                pltpu.VMEM((NG, M, GD), BF16),
                pltpu.VMEM((NG, M, GD), BF16),
                pltpu.SemaphoreType.DMA((6,)),
                pltpu.SemaphoreType.DMA((R,)),
                pltpu.SemaphoreType.DMA((R,)),
                pltpu.SemaphoreType.DMA((WO_CH,)),
                pltpu.SemaphoreType.DMA((WD_CH,)),
                pltpu.SemaphoreType.DMA((2,)),
            ],
            compiler_params=pltpu.CompilerParams(vmem_limit_bytes=110 * 1024 * 1024),
        )(A_x, c, kt, vt, A_wq, A_wo, B_w_gate, B_w_up, B_w_down, w_mod)
    return fn


_impl = build(G=2, R=4, WO_CH=4, WD_CH=2)


@jax.jit
def pallas_adaLN_cond__sliding_block_cached__glu_gated_bilinear__decode_kernel(
    A_x: jax.Array,
    A_k_cache: jax.Array,
    A_v_cache: jax.Array,
    A_wq: jax.Array,
    A_wo: jax.Array,
    B_x: jax.Array,
    B_w_gate: jax.Array,
    B_w_up: jax.Array,
    B_w_down: jax.Array,
    c: jax.Array,
    w_mod: jax.Array,
):
    return _impl(A_x, A_k_cache, A_v_cache, A_wq, A_wo, B_x, B_w_gate, B_w_up, B_w_down, c, w_mod)
```

```python
import jax
import jax.numpy as jnp
from jax import lax
import jax.experimental.pallas as pl
import jax.experimental.pallas.tpu as pltpu

F32 = jnp.float32
BF16 = jnp.bfloat16

D, H, DH, F = 640, 32, 192, 1536
G = 2
GD = G * DH
NG = H // G
M = 8
LANE = 128
HI, LO = 0, 1

S_K, S_V, S_QO, S_OTH, S_A, S_B = range(6)
NSEM = 6


def _layernorm(x, eps=1e-5):
    m = jnp.mean(x, axis=-1, keepdims=True)
    xc = x - m
    v = jnp.mean(xc * xc, axis=-1, keepdims=True)
    return xc * lax.rsqrt(v + eps)


def _dot(a, b):
    return jnp.dot(a, b, preferred_element_type=F32)


def _dot_nt(a, b):
    return lax.dot_general(a, b, (((1,), (1,)), ((), ())), preferred_element_type=F32)


def build(debug=False, checks=False, TPT=2, WDF=320, WDB=256, compute=True):
    scale = DH ** -0.5

    def make(Sk, W):
        NT = W // LANE
        W0 = Sk - W

        def kernel(x_hbm, c_hbm, k_hbm, v_hbm, wq_hbm, wo_hbm, wg_hbm, wu_hbm, wd_hbm, wm_hbm,
                   o_ref,
                   x_v, c_v, wm_v, wq_v, wo_v, wg_v, wu_v, wd_v, kbuf, vbuf, q_s, acc_s, s_s, sem):
            def copy(src, dst, s):
                return pltpu.make_async_copy(src, dst, sem.at[s])

            def wait_all(dst, s):
                copy(dst, dst, s).wait()

            def row0(g, mult, off):
                r = g * mult + off
                return r if isinstance(r, int) else pl.multiple_of(r, 8)

            def k_piece(g, j):
                return copy(k_hbm.at[pl.ds(row0(g, GD, 0), GD), pl.ds(W0 + j * LANE, LANE)],
                            kbuf.at[g % 2, :, pl.ds(j * LANE, LANE)], S_K)

            def v_piece(g, j):
                return copy(v_hbm.at[pl.ds(row0(g, GD, 0), GD), pl.ds(W0 + j * LANE, LANE)],
                            vbuf.at[g % 2, :, pl.ds(j * LANE, LANE)], S_V)

            def wm_piece(i):
                return copy(wm_hbm.at[pl.ds(32 * i, 32), pl.ds(0, 2 * D)],
                            wm_v.at[pl.ds(32 * i, 32), pl.ds(0, 2 * D)], S_V)

            def q_piece(g, i):
                c0 = g * GD
                c0 = c0 if isinstance(c0, int) else pl.multiple_of(c0, LANE)
                return copy(wq_hbm.at[pl.ds(32 * i, 32), pl.ds(c0, GD)], wq_v.at[pl.ds(32 * i, 32), :], S_QO)

            def o_piece(g, i):
                return copy(wo_hbm.at[pl.ds(row0(g, GD, 16 * i), 16), :], wo_v.at[pl.ds(16 * i, 16), :], S_QO)

            def oth_piece(n, i):
                kind, r = i % 4, row0(n, 40, 8 * (i // 4))
                if kind == 0:
                    return copy(wg_hbm.at[pl.ds(r, 8), :], wg_v.at[pl.ds(r, 8), :], S_OTH)
                if kind == 1:
                    return copy(wu_hbm.at[pl.ds(r, 8), :], wu_v.at[pl.ds(r, 8), :], S_OTH)
                c0 = 2 * D * (kind - 1)
                return copy(wm_hbm.at[pl.ds(r, 8), pl.ds(c0, 2 * D)], wm_v.at[pl.ds(r, 8), pl.ds(c0, 2 * D)], S_OTH)

            def d_piece(i, s):
                return copy(wd_hbm.at[pl.ds(16 * i, 16), :], wd_v.at[pl.ds(16 * i, 16), :], s)

            cp_c = copy(c_hbm, c_v, S_A)
            cp_x = copy(x_hbm, x_v, S_B)
            cp_da = copy(wd_hbm.at[pl.ds(WDF, F - WDB - WDF), :], wd_v.at[pl.ds(WDF, F - WDB - WDF), :], S_A)
            cp_db = copy(wd_hbm.at[pl.ds(F - WDB, WDB), :], wd_v.at[pl.ds(F - WDB, WDB), :], S_B)
            n_d0 = min(12, WDF // 16)
            n_d1 = WDF // 16 - n_d0

            def phase(waits, bulk, small, work):
                for j in range(len(waits)):
                    waits[j].wait()
                    for cp in bulk.get(j, ()):
                        cp.start(priority=LO)
                    for cp in small.get(j, ()):
                        cp.start(priority=HI)
                    if compute:
                        for fn in work.get(j, ()):
                            fn()

            row = lax.broadcasted_iota(jnp.int32, (M, GD), 0)
            col = lax.broadcasted_iota(jnp.int32, (M, GD), 1)
            diag = (col >= row * DH) & (col < (row + 1) * DH)
            st = {}

            def qk_slice(g, t):
                def fn():
                    c0 = t * TPT * LANE
                    s = _dot(q_s[...], kbuf[g % 2, :, c0:c0 + TPT * LANE])
                    s_s[:, c0:c0 + TPT * LANE] = s
                    mx = s[:, 0:LANE]
                    for u in range(1, TPT):
                        mx = jnp.maximum(mx, s[:, u * LANE:(u + 1) * LANE])
                    st['mx'] = mx if t == 0 else jnp.maximum(st['mx'], mx)
                return fn

            def max_fin():
                st['m'] = jnp.max(st['mx'], axis=-1, keepdims=True)

            def pv_slice(g, t, tpt=TPT):
                def fn():
                    c0 = t * tpt * LANE
                    p = jnp.exp((s_s[:, c0:c0 + tpt * LANE] - st['m']) * scale)
                    ps = p[:, 0:LANE]
                    for u in range(1, tpt):
                        ps = ps + p[:, u * LANE:(u + 1) * LANE]
                    o = _dot_nt(p.astype(BF16), vbuf[g % 2, :, c0:c0 + tpt * LANE])
                    st['l'] = ps if t == 0 else st['l'] + ps
                    st['o'] = o if t == 0 else o + st['o']
                return fn

            def pv_fin():
                l = jnp.sum(st['l'], axis=-1, keepdims=True)
                st['ob'] = jnp.where(diag, st['o'] / l, 0.0).astype(BF16)

            def wo_slice(n):
                def fn():
                    cs = slice(n * LANE, (n + 1) * LANE)
                    acc_s[:, cs] = _dot(st['ob'], wo_v[:, cs]) + acc_s[:, cs]
                return fn

            def qp_slice(n):
                def fn():
                    cs = slice(n * LANE, (n + 1) * LANE)
                    q = _dot(st['h'], wq_v[:, cs])
                    q_s[:, cs] = jnp.where(diag[:, cs], q, 0.0).astype(BF16)
                return fn

            def mod_slice(c0, n):
                def fn():
                    st.setdefault('mod', {})[c0] = _dot(st['sc'], wm_v[:, c0:c0 + n])
                return fn

            def mod_part(i):
                return jnp.concatenate([st['mod'][c] for c in range(i * D, (i + 1) * D, LANE)], axis=1)

            cp_c.start(priority=HI)
            cp_x.start(priority=HI)
            for i in range(20):
                wm_piece(i).start(priority=LO)
            for j in range(NT):
                k_piece(0, j).start(priority=LO)

            def prep():
                c = c_v[...].astype(F32)
                sc = c * (1.0 / (1.0 + jnp.exp(-c)))
                st['sc'] = jnp.broadcast_to(sc, (M, D)).astype(BF16)
                x = x_v[...].reshape(1, D).astype(F32)
                st['x'] = jnp.broadcast_to(x, (M, D))
                st['lnx'] = _layernorm(st['x'])
                acc_s[...] = jnp.zeros((M, D), F32)

            phase([wm_piece(i) for i in range(20)], {}, {i: [q_piece(0, i)] for i in range(20)},
                  {2: [cp_c.wait, cp_x.wait, prep]} if compute else {})
            if not compute:
                cp_c.wait(); cp_x.wait()

            def make_h():
                st['h'] = (st['lnx'] * (1.0 + mod_part(1)) + mod_part(0)).astype(BF16)

            def wait_q():
                wait_all(wq_v, S_QO)

            work = {t: [mod_slice(t * LANE, LANE)] for t in range(10)}
            work[11] = [make_h]
            work[13] = [qp_slice(0)]
            work[14] = [qp_slice(1)]
            work[15] = [qp_slice(2)]
            small = {i: [oth_piece(0, i)] for i in range(20)}
            for i in range(n_d0):
                small[20 + i] = [d_piece(i, S_OTH)]
            waits = [k_piece(0, j) for j in range(NT)]
            phase(waits[:12], {j: [v_piece(0, j)] for j in range(12)}, small, work)
            wait_q()
            phase(waits[12:], {j - 12: [v_piece(0, j)] for j in range(12, NT)},
                  {j - 12: v for j, v in small.items() if j >= 12}, {j - 12: v for j, v in work.items() if j >= 12})

            nsl = NT // TPT
            h = st.get('h')

            def body(g, carry):
                st['h'] = h
                qo = [q_piece(g + 1, i) for i in range(20)] + [o_piece(g, i) for i in range(24)]
                work = {t: [qk_slice(g, t)] for t in range(nsl)}
                work[nsl] = [max_fin]
                phase([v_piece(g, j) for j in range(NT)], {j: [k_piece(g + 1, j)] for j in range(NT)},
                      {j: [qo[j]] for j in range(NT)}, work)
                small = {j: [qo[NT + j]] for j in range(12)}
                for i in range(20):
                    small[12 + i] = [oth_piece(g + 1, i)]
                work = {t: [pv_slice(g, t)] for t in range(nsl)}
                work[nsl] = [pv_fin]
                tw = max(nsl + 2, 18)
                for n in range(5):
                    work[tw + n] = [wo_slice(n)]
                for n in range(3):
                    work[tw + 5 + n] = [qp_slice(n)]
                waits = [k_piece(g + 1, j) for j in range(NT)]
                phase(waits[:tw], {j: [v_piece(g + 1, j)] for j in range(tw)}, small, work)
                wait_all(wq_v, S_QO)
                wait_all(wo_v, S_QO)
                phase(waits[tw:], {j - tw: [v_piece(g + 1, j)] for j in range(tw, NT)},
                      {j - tw: v for j, v in small.items() if j >= tw},
                      {j - tw: v for j, v in work.items() if j >= tw})
                return carry

            lax.fori_loop(0, NG - 1, body, 0)

            g = NG - 1
            small = {i: [o_piece(g, i)] for i in range(24)}
            for i in range(n_d1):
                small[24 + i] = [d_piece(n_d0 + i, S_QO)]
            work = {t: [qk_slice(g, t)] for t in range(nsl)}
            work[nsl] = [max_fin]
            waits = [v_piece(g, j) for j in range(NT)]
            phase(waits[:8], {0: [cp_da, cp_db]}, small, work)
            wait_all(wg_v, S_OTH)
            wait_all(wu_v, S_OTH)
            wait_all(wm_v.at[:, pl.ds(2 * D, 4 * D)], S_OTH)
            if n_d0:
                wait_all(wd_v.at[pl.ds(0, 16 * n_d0), :], S_OTH)
            for t in range(20):
                work.setdefault(12 + t, []).append(mod_slice(2 * D + t * LANE, LANE))
            phase(waits[8:], {}, {j - 8: v for j, v in small.items() if j >= 8},
                  {j - 8: v for j, v in work.items() if j >= 8})

            if compute:
                pv_slice(g, 0, NT)()
                pv_fin()
            wait_all(wo_v, S_QO)
            if n_d1:
                wait_all(wd_v.at[pl.ds(16 * n_d0, 16 * n_d1), :], S_QO)
            if not compute:
                cp_da.wait(); cp_db.wait()
                o_ref[...] = x_v[...]
                return
            acc = _dot(st['ob'], wo_v[...]) + acc_s[...]
            attn = jnp.sum(acc, axis=0, keepdims=True)
            x1 = st['x'] + mod_part(2) * attn
            h2 = (_layernorm(x1) * (1.0 + mod_part(4)) + mod_part(3)).astype(BF16)
            gg = _dot(h2, wg_v[...])
            uu = _dot(h2, wu_v[...])
            hh = (gg * uu).astype(BF16)
            cp_da.wait()
            ffn = _dot(hh[:, :F - WDB], wd_v[0:F - WDB, :])
            cp_db.wait()
            ffn = _dot(hh[:, F - WDB:], wd_v[F - WDB:F, :]) + ffn
            out = x1 + mod_part(5) * ffn
            if debug:
                o_ref[0] = out[0:1]
                o_ref[1] = attn
                o_ref[2] = ffn[0:1]
            else:
                o_ref[...] = out[0:1].reshape(1, 1, D).astype(o_ref.dtype)
        return kernel

    @jax.jit
    def fn(A_x, A_k_cache, A_v_cache, A_wq, A_wo, B_x, B_w_gate, B_w_up, B_w_down, c, w_mod):
        Sk = A_k_cache.shape[2]
        W = min(4096, max(256, Sk // 4))
        kt = jnp.swapaxes(A_k_cache, 2, 3).reshape(H * DH, Sk)
        vt = jnp.swapaxes(A_v_cache, 2, 3).reshape(H * DH, Sk)
        any_spec = pl.BlockSpec(memory_space=pl.ANY)
        out_shape = jax.ShapeDtypeStruct((3, 1, D), F32) if debug else jax.ShapeDtypeStruct((1, 1, D), A_x.dtype)
        return pl.pallas_call(
            make(Sk, W),
            out_shape=out_shape,
            in_specs=[any_spec] * 10,
            scratch_shapes=[
                pltpu.VMEM((1, 1, D), BF16),
                pltpu.VMEM((1, D), BF16),
                pltpu.VMEM((D, 6 * D), BF16),
                pltpu.VMEM((D, GD), BF16),
                pltpu.VMEM((GD, D), BF16),
                pltpu.VMEM((D, F), BF16),
                pltpu.VMEM((D, F), BF16),
                pltpu.VMEM((F, D), BF16),
                pltpu.VMEM((2, GD, W), BF16),
                pltpu.VMEM((2, GD, W), BF16),
                pltpu.VMEM((M, GD), BF16),
                pltpu.VMEM((M, D), F32),
                pltpu.VMEM((M, W), F32),
                pltpu.SemaphoreType.DMA((NSEM,)),
            ],
            compiler_params=pltpu.CompilerParams(vmem_limit_bytes=64 * 1024 * 1024,
                                                 disable_bounds_checks=not checks,
                                                 disable_semaphore_checks=not checks),
        )(A_x, c, kt, vt, A_wq, A_wo, B_w_gate, B_w_up, B_w_down, w_mod)
    return fn


_impl = build(WDF=0, checks=True)


@jax.jit
def pallas_adaLN_cond__sliding_block_cached__glu_gated_bilinear__decode_kernel(
    A_x: jax.Array,
    A_k_cache: jax.Array,
    A_v_cache: jax.Array,
    A_wq: jax.Array,
    A_wo: jax.Array,
    B_x: jax.Array,
    B_w_gate: jax.Array,
    B_w_up: jax.Array,
    B_w_down: jax.Array,
    c: jax.Array,
    w_mod: jax.Array,
):
    return _impl(A_x, A_k_cache, A_v_cache, A_wq, A_wo, B_x, B_w_gate, B_w_up, B_w_down, c, w_mod)
```

```python
import jax
import jax.numpy as jnp
from jax import lax
import jax.experimental.pallas as pl
import jax.experimental.pallas.tpu as pltpu

F32 = jnp.float32
BF16 = jnp.bfloat16

D, H, DH, F = 640, 32, 192, 1536
G = 2
GD = G * DH
NG = H // G
M = 8
LANE = 128
HI, LO = 0, 1

S_K, S_QO, S_OTH, S_A, S_B, S_V = range(6)


def _layernorm(x, eps=1e-5):
    m = jnp.mean(x, axis=-1, keepdims=True)
    xc = x - m
    v = jnp.mean(xc * xc, axis=-1, keepdims=True)
    return xc * lax.rsqrt(v + eps)


def _dot(a, b):
    return jnp.dot(a, b, preferred_element_type=F32)


def _dot_nt(a, b):
    return lax.dot_general(a, b, (((1,), (1,)), ((), ())), preferred_element_type=F32)


def build(debug=False, checks=False, WDF=320, WDB=256, compute=True, notail=False,
          VSPLIT=(12, 24), LASTQK=3, wm_cols=False):
    scale = DH ** -0.5
    NSEM = S_V + len(VSPLIT) + 1

    def make(Sk, W):
        NT = W // LANE
        W0 = Sk - W
        vbounds = (0,) + tuple(VSPLIT) + (NT,)

        def vsem(j):
            return S_V + sum(j >= b for b in VSPLIT)

        def kernel(x_hbm, c_hbm, k_hbm, v_hbm, wq_hbm, wo_hbm, wg_hbm, wu_hbm, wd_hbm, wm_hbm,
                   o_ref,
                   x_v, c_v, wm_v, wq_v, wo_v, wg_v, wu_v, wd_v, kbuf, vbuf, q_s, acc_s, s_s, sem):
            def copy(src, dst, s):
                return pltpu.make_async_copy(src, dst, sem.at[s])

            def wait_all(dst, s):
                return lambda: copy(dst, dst, s).wait()

            def row0(g, mult, off):
                r = g * mult + off
                return r if isinstance(r, int) else pl.multiple_of(r, 8)

            def k_piece(g, j):
                return copy(k_hbm.at[pl.ds(row0(g, GD, 0), GD), pl.ds(W0 + j * LANE, LANE)],
                            kbuf.at[g % 2, :, pl.ds(j * LANE, LANE)], S_K)

            def v_piece(g, j):
                return copy(v_hbm.at[pl.ds(row0(g, GD, 0), GD), pl.ds(W0 + j * LANE, LANE)],
                            vbuf.at[g % 2, :, pl.ds(j * LANE, LANE)], vsem(j))

            if wm_cols:
                NWM = 60
                def wm_piece(i):
                    r, c0 = 320 * (i % 2), LANE * (i // 2)
                    return copy(wm_hbm.at[pl.ds(r, 320), pl.ds(c0, LANE)], wm_v.at[pl.ds(r, 320), pl.ds(c0, LANE)], S_V)
            else:
                NWM = 40
                def wm_piece(i):
                    return copy(wm_hbm.at[pl.ds(16 * i, 16), :], wm_v.at[pl.ds(16 * i, 16), :], S_V)

            def q_piece(g, i, rows=32):
                c0 = g * GD
                c0 = c0 if isinstance(c0, int) else pl.multiple_of(c0, LANE)
                return copy(wq_hbm.at[pl.ds(rows * i, rows), pl.ds(c0, GD)], wq_v.at[pl.ds(rows * i, rows), :], S_QO)

            def o_piece(g, i):
                return copy(wo_hbm.at[pl.ds(row0(g, GD, 16 * i), 16), :], wo_v.at[pl.ds(16 * i, 16), :], S_QO)

            def oth_piece(n, i):
                src, dst = ((wg_hbm, wg_v), (wu_hbm, wu_v))[i % 2]
                r, c0 = row0(n, 40, 8 * (i // 4)), (F // 2) * ((i // 2) % 2)
                return copy(src.at[pl.ds(r, 8), pl.ds(c0, F // 2)], dst.at[pl.ds(r, 8), pl.ds(c0, F // 2)], S_OTH)

            def d_piece(i):
                return copy(wd_hbm.at[pl.ds(16 * i, 16), :], wd_v.at[pl.ds(16 * i, 16), :], S_OTH)

            def cp_c():
                return copy(c_hbm, c_v, S_A)

            def cp_x():
                return copy(x_hbm, x_v, S_B)

            def cp_da():
                return copy(wd_hbm.at[pl.ds(WDF, F - WDB - WDF), :], wd_v.at[pl.ds(WDF, F - WDB - WDF), :], S_A)

            def cp_db():
                return copy(wd_hbm.at[pl.ds(F - WDB, WDB), :], wd_v.at[pl.ds(F - WDB, WDB), :], S_B)

            n_d0 = min(12, WDF // 16)
            n_d1 = WDF // 16 - n_d0

            def phase(n, wait, bulk, small, work, sync=None):
                for j in range(n):
                    wait(j).wait()
                    for cp in bulk(j):
                        cp.start(priority=LO)
                    for cp in small(j):
                        cp.start(priority=HI)
                    for fn in (sync or {}).get(j, ()):
                        fn()
                    if compute:
                        for fn in work.get(j, ()):
                            fn()

            row = lax.broadcasted_iota(jnp.int32, (M, GD), 0)
            col = lax.broadcasted_iota(jnp.int32, (M, GD), 1)
            diag = (col >= row * DH) & (col < (row + 1) * DH)
            st = {}

            def qk_slice(g, t0, t1):
                def fn():
                    cs = slice(t0 * LANE, t1 * LANE)
                    s = _dot(q_s[...], kbuf[g % 2, :, cs])
                    s_s[:, cs] = s
                    mx = s[:, 0:LANE]
                    for u in range(1, t1 - t0):
                        mx = jnp.maximum(mx, s[:, u * LANE:(u + 1) * LANE])
                    st['mx'] = mx if t0 == 0 else jnp.maximum(st['mx'], mx)
                return fn

            def max_fin():
                st['m'] = jnp.max(st['mx'], axis=-1, keepdims=True)

            def pv_slice(g, t0, t1):
                def fn():
                    cs = slice(t0 * LANE, t1 * LANE)
                    p = jnp.exp((s_s[:, cs] - st['m']) * scale)
                    ps = p[:, 0:LANE]
                    for u in range(1, t1 - t0):
                        ps = ps + p[:, u * LANE:(u + 1) * LANE]
                    o = _dot_nt(p.astype(BF16), vbuf[g % 2, :, cs])
                    st['l'] = ps if t0 == 0 else st['l'] + ps
                    st['o'] = o if t0 == 0 else o + st['o']
                return fn

            def pv_fin():
                l = jnp.sum(st['l'], axis=-1, keepdims=True)
                st['ob'] = jnp.where(diag, st['o'] / l, 0.0).astype(BF16)

            def wo_slice(n0, n1):
                def fn():
                    cs = slice(n0 * LANE, n1 * LANE)
                    acc_s[:, cs] = _dot(st['ob'], wo_v[:, cs]) + acc_s[:, cs]
                return fn

            def qp_slice(n):
                def fn():
                    cs = slice(n * LANE, (n + 1) * LANE)
                    q = _dot(st['h'], wq_v[:, cs])
                    q_s[:, cs] = jnp.where(diag[:, cs], q, 0.0).astype(BF16)
                return fn

            def mod_slice(t):
                def fn():
                    st.setdefault('mod', {})[t] = _dot(st['sc'], wm_v[:, t * LANE:(t + 1) * LANE])
                return fn

            def mod_part(i):
                n = D // LANE
                return jnp.concatenate([st['mod'][t] for t in range(i * n, (i + 1) * n)], axis=1)

            none = lambda j: ()

            cp_c().start(priority=HI)
            cp_x().start(priority=HI)
            for i in range(NWM):
                wm_piece(i).start(priority=LO)

            def prep():
                c = c_v[...].astype(F32)
                sc = c * (1.0 / (1.0 + jnp.exp(-c)))
                st['sc'] = jnp.broadcast_to(sc, (M, D)).astype(BF16)
                x = x_v[...].reshape(1, D).astype(F32)
                st['x'] = jnp.broadcast_to(x, (M, D))
                st['lnx'] = _layernorm(st['x'])
                acc_s[...] = jnp.zeros((M, D), F32)

            hq = {i * NWM // 40: i for i in range(40)}
            phase(NWM, wm_piece, lambda j: [k_piece(0, j)] if j < NT else [],
                  lambda j: [q_piece(0, hq[j], 16)] if j in hq else [],
                  {2: [prep]}, {2: [lambda: cp_c().wait(), lambda: cp_x().wait()]})

            def make_h():
                st['h'] = (st['lnx'] * (1.0 + mod_part(1)) + mod_part(0)).astype(BF16)

            work = {t: [mod_slice(t)] for t in range(30)}
            work[10].append(make_h)
            for n in range(3):
                work[12 + n].append(qp_slice(n))
            phase(NT, lambda j: k_piece(0, j), lambda j: [v_piece(0, j)],
                  lambda j: [oth_piece(0, j)] if j < 20 else ([d_piece(j - 20)] if j - 20 < n_d0 else []),
                  work, {12: [wait_all(wq_v, S_QO)]})

            keep = {k: st[k] for k in ('h',) if k in st}

            def body(g, carry):
                st.update(keep)

                def qo(i):
                    return q_piece(g + 1, i) if i < 20 else o_piece(g, i - 20)

                work = {t: [qk_slice(g, 2 * t, 2 * t + 2)] for t in range(16)}
                work[16] = [max_fin]
                for t in range(15):
                    work[17 + t] = [pv_slice(g, t, t + 1)]
                phase(NT, lambda j: v_piece(g, j), lambda j: [k_piece(g + 1, j)], lambda j: [qo(j)], work)
                work = {t: [pv_slice(g, 15 + t, 16 + t)] for t in range(17)}
                work[17] = [pv_fin]
                work[19] = [wo_slice(0, 2)]
                work[20] = [wo_slice(2, 4)]
                work[21] = [wo_slice(4, 5)]
                for n in range(3):
                    work[22 + n] = [qp_slice(n)]
                phase(NT, lambda j: k_piece(g + 1, j), lambda j: [v_piece(g + 1, j)],
                      lambda j: [qo(NT + j)] if j < 12 else [oth_piece(g + 1, j - 12)], work,
                      {19: [wait_all(wq_v, S_QO), wait_all(wo_v, S_QO)]})
                return carry

            lax.fori_loop(0, NG - 1, body, 0)

            g = NG - 1
            work = {}
            t, j = 0, 0
            while t < NT:
                work[j] = [qk_slice(g, t, min(NT, t + LASTQK))]
                t += LASTQK
                j += 1
            work[j] = [max_fin]
            j += 1
            t = 0
            last = vbounds[-2]
            while t < last and j < NT:
                avail = max(b for b in vbounds if b <= j + 1)
                rem_ticks = NT - 2 - j
                n = 1 if (last - t) <= rem_ticks else 2
                n = min(n, avail - t)
                if n > 0:
                    work[j] = [pv_slice(g, t, t + n)]
                    t += n
                j += 1
            phase(NT, lambda j: v_piece(g, j), lambda j: [cp_da(), cp_db()] if j == 0 else [],
                  lambda j: [o_piece(g, j)] if j < 24 else ([d_piece(n_d0 + j - 24)] if j - 24 < n_d1 else []),
                  work)

            if compute and not notail:
                pv_slice(g, t, NT)()
                pv_fin()
            wait_all(wo_v, S_QO)()
            if not compute or notail:
                wait_all(wg_v, S_OTH)()
                wait_all(wu_v, S_OTH)()
                if WDF:
                    wait_all(wd_v.at[pl.ds(0, WDF), :], S_OTH)()
                cp_da().wait(); cp_db().wait()
                if notail:
                    r = (acc_s[...] + mod_part(2) + mod_part(3) + mod_part(4) + mod_part(5) + st['m'] + st['o'][:, 0:1] + st['l'][:, 0:1])[0:1]
                    o_ref[...] = r.reshape(1, 1, D).astype(o_ref.dtype)
                else:
                    o_ref[...] = x_v[...]
                return
            wait_all(wg_v, S_OTH)()
            wait_all(wu_v, S_OTH)()
            if WDF:
                wait_all(wd_v.at[pl.ds(0, WDF), :], S_OTH)()
            acc = _dot(st['ob'], wo_v[...]) + acc_s[...]
            attn = jnp.sum(acc, axis=0, keepdims=True)
            x1 = st['x'] + mod_part(2) * attn
            h2 = (_layernorm(x1) * (1.0 + mod_part(4)) + mod_part(3)).astype(BF16)
            gg = _dot(h2, wg_v[...])
            uu = _dot(h2, wu_v[...])
            hh = (gg * uu).astype(BF16)
            cp_da().wait()
            ffn = _dot(hh[:, :F - WDB], wd_v[0:F - WDB, :])
            cp_db().wait()
            ffn = _dot(hh[:, F - WDB:], wd_v[F - WDB:F, :]) + ffn
            out = x1 + mod_part(5) * ffn
            if debug:
                o_ref[0] = out[0:1]
                o_ref[1] = attn
                o_ref[2] = ffn[0:1]
            else:
                o_ref[...] = out[0:1].reshape(1, 1, D).astype(o_ref.dtype)
        return kernel

    @jax.jit
    def fn(A_x, A_k_cache, A_v_cache, A_wq, A_wo, B_x, B_w_gate, B_w_up, B_w_down, c, w_mod):
        Sk = A_k_cache.shape[2]
        W = min(4096, max(256, Sk // 4))
        kt = jnp.swapaxes(A_k_cache, 2, 3).reshape(H * DH, Sk)
        vt = jnp.swapaxes(A_v_cache, 2, 3).reshape(H * DH, Sk)
        any_spec = pl.BlockSpec(memory_space=pl.ANY)
        out_shape = jax.ShapeDtypeStruct((3, 1, D), F32) if debug else jax.ShapeDtypeStruct((1, 1, D), A_x.dtype)
        return pl.pallas_call(
            make(Sk, W),
            out_shape=out_shape,
            in_specs=[any_spec] * 10,
            scratch_shapes=[
                pltpu.VMEM((1, 1, D), BF16),
                pltpu.VMEM((1, D), BF16),
                pltpu.VMEM((D, 6 * D), BF16),
                pltpu.VMEM((D, GD), BF16),
                pltpu.VMEM((GD, D), BF16),
                pltpu.VMEM((D, F), BF16),
                pltpu.VMEM((D, F), BF16),
                pltpu.VMEM((F, D), BF16),
                pltpu.VMEM((2, GD, W), BF16),
                pltpu.VMEM((2, GD, W), BF16),
                pltpu.VMEM((M, GD), BF16),
                pltpu.VMEM((M, D), F32),
                pltpu.VMEM((M, W), F32),
                pltpu.SemaphoreType.DMA((NSEM,)),
            ],
            compiler_params=pltpu.CompilerParams(vmem_limit_bytes=64 * 1024 * 1024,
                                                 disable_bounds_checks=not checks,
                                                 disable_semaphore_checks=not checks),
        )(A_x, c, kt, vt, A_wq, A_wo, B_w_gate, B_w_up, B_w_down, w_mod)
    return fn


_impl = build(WDF=192)


@jax.jit
def pallas_adaLN_cond__sliding_block_cached__glu_gated_bilinear__decode_kernel(
    A_x: jax.Array,
    A_k_cache: jax.Array,
    A_v_cache: jax.Array,
    A_wq: jax.Array,
    A_wo: jax.Array,
    B_x: jax.Array,
    B_w_gate: jax.Array,
    B_w_up: jax.Array,
    B_w_down: jax.Array,
    c: jax.Array,
    w_mod: jax.Array,
):
    return _impl(A_x, A_k_cache, A_v_cache, A_wq, A_wo, B_x, B_w_gate, B_w_up, B_w_down, c, w_mod)
```

```python
import jax
import jax.numpy as jnp
from jax import lax
import jax.experimental.pallas as pl
import jax.experimental.pallas.tpu as pltpu

F32 = jnp.float32
BF16 = jnp.bfloat16

D, H, DH, F = 640, 32, 192, 1536
G = 2
GD = G * DH
NG = H // G
M = 8
LANE = 128
NS = D // LANE
HI, LO = 0, 1
CR = 48

S_K, S_O, S_OTH, S_A, S_B, S_V = range(6)


def _layernorm(x, eps=1e-5):
    m = jnp.mean(x, axis=-1, keepdims=True)
    xc = x - m
    v = jnp.mean(xc * xc, axis=-1, keepdims=True)
    return xc * lax.rsqrt(v + eps)


def _dot(a, b):
    return jnp.dot(a, b, preferred_element_type=F32)


def _dot_nt(a, b):
    return lax.dot_general(a, b, (((1,), (1,)), ((), ())), preferred_element_type=F32)


def _spread(items, n):
    out = [[] for _ in range(n)]
    for i, it in enumerate(items):
        out[i * n // len(items)].append(it)
    return out


def build(debug=False, checks=False, WDF=192, WDB=256, compute=True, notail=False,
          VSPLIT=(12, 24), LASTQK=3, LA=32, QPT=2, dummy=0, QK=(4, 2), PV=(2, 2), QP=(3, 2), MOD=(2, 5)):
    scale = DH ** -0.5
    NSEM = S_V + len(VSPLIT) + 1

    def make(Sk, W):
        NT = W // LANE
        W0 = Sk - W
        vbounds = (0,) + tuple(VSPLIT) + (NT,)
        CARVE0 = 18

        def vsem(j):
            return S_V + sum(j >= b for b in VSPLIT)

        def kernel(x_hbm, c_hbm, k_hbm, v_hbm, wq_hbm, wo_hbm, wg_hbm, wu_hbm, wd_hbm, wm_hbm,
                   o_ref,
                   x_v, c_v, wm_v, wq_v, wo_v, wg_v, wu_v, wd_v, kbuf, vbuf, q_s, acc_s, s_s, sem):
            def copy(src, dst, s):
                return pltpu.make_async_copy(src, dst, sem.at[s])

            def wait_all(dst, s):
                return lambda: copy(dst, dst, s).wait()

            def row0(g, mult, off):
                r = g * mult + off
                return r if isinstance(r, int) else pl.multiple_of(r, 8)

            def k_piece(g, j):
                return lambda: copy(k_hbm.at[pl.ds(row0(g, GD, 0), GD), pl.ds(W0 + j * LANE, LANE)],
                                    kbuf.at[g % 2, :, pl.ds(j * LANE, LANE)], S_K)

            def v_rows(g, j, r0, nr):
                return lambda: copy(v_hbm.at[pl.ds(row0(g, GD, r0), nr), pl.ds(W0 + j * LANE, LANE)],
                                    vbuf.at[g % 2, pl.ds(r0, nr), pl.ds(j * LANE, LANE)], vsem(j))

            def v_bulk(g, j):
                return v_rows(g, j, 0, GD - CR if j >= CARVE0 else GD)

            def v_small(g, j):
                return [v_rows(g, j, GD - CR, CR)] if j >= CARVE0 else []

            def streams(src, dst, r, c, nc, s):
                return lambda: copy(src.at[:, pl.ds(r, 8), pl.ds(c, nc)], dst.at[:, pl.ds(r, 8), pl.ds(c, nc)], s)

            def rect(src, dst, r, nr, c, nc, s):
                return lambda: copy(src.at[pl.ds(r, nr), pl.ds(c, nc)], dst.at[pl.ds(r, nr), pl.ds(c, nc)], s)

            def o_pieces(g):
                return [(lambda r=r, c=c: copy(wo_hbm.at[pl.ds(row0(g, GD, r), 48), pl.ds(c, LANE)],
                                               wo_v.at[pl.ds(r, 48), pl.ds(c, LANE)], S_O))
                        for r in range(0, GD, 48) for c in range(0, D, LANE)]

            def u_pieces(n):
                return [rect(wu_hbm, wu_v, row0(n, 40, r), 8, c, F // 2, S_OTH)
                        for r in range(0, 40, 8) for c in (0, F // 2)]

            def d_pieces(r0, r1):
                return [rect(wd_hbm, wd_v, r, 8, 0, D, S_OTH) for r in range(r0, r1, 8)]

            cp_c = lambda: copy(c_hbm, c_v, S_A)
            cp_x = lambda: copy(x_hbm, x_v, S_B)
            cp_da = rect(wd_hbm, wd_v, WDF, F - WDB - WDF, 0, D, S_A)
            cp_db = rect(wd_hbm, wd_v, F - WDB, WDB, 0, D, S_B)
            WD0 = min(WDF, 64)

            def phase(waits, bulk, small, work, sync=None):
                for j in range(len(waits)):
                    for mk in waits[j]:
                        mk().wait()
                    for mk in bulk[j]:
                        mk().start(priority=LO)
                    for mk in small[j]:
                        mk().start(priority=HI)
                    for fn in (sync or {}).get(j, ()):
                        fn()
                    if compute:
                        for fn in work.get(j, ()):
                            fn()
                    elif dummy and work.get(j):
                        a = acc_s[:, 0:LANE]
                        for u in range(dummy):
                            a = a * 1.0001 + float(u + j)
                        acc_s[:, 0:LANE] = a

            row = lax.broadcasted_iota(jnp.int32, (M, GD), 0)
            col = lax.broadcasted_iota(jnp.int32, (M, GD), 1)
            diag = (col >= row * DH) & (col < (row + 1) * DH)
            st = {}

            def qk_slice(g, t0, t1):
                def fn():
                    cs = slice(t0 * LANE, t1 * LANE)
                    s = _dot(q_s[g], kbuf[g % 2, :, cs])
                    s_s[:, cs] = s
                    mx = s[:, 0:LANE]
                    for u in range(1, t1 - t0):
                        mx = jnp.maximum(mx, s[:, u * LANE:(u + 1) * LANE])
                    st['mx'] = mx if t0 == 0 else jnp.maximum(st['mx'], mx)
                return fn

            def max_fin():
                st['m'] = jnp.max(st['mx'], axis=-1, keepdims=True)

            def pv_slice(g, t0, t1):
                def fn():
                    cs = slice(t0 * LANE, t1 * LANE)
                    p = jnp.exp((s_s[:, cs] - st['m']) * scale)
                    ps = p[:, 0:LANE]
                    for u in range(1, t1 - t0):
                        ps = ps + p[:, u * LANE:(u + 1) * LANE]
                    o = _dot_nt(p.astype(BF16), vbuf[g % 2, :, cs])
                    st['l'] = ps if t0 == 0 else st['l'] + ps
                    st['o'] = o if t0 == 0 else o + st['o']
                return fn

            def pv_fin():
                l = jnp.sum(st['l'], axis=-1, keepdims=True)
                st['ob'] = jnp.where(diag, st['o'] / l, 0.0).astype(BF16)

            def wo_slice(n0, n1):
                def fn():
                    cs = slice(n0 * LANE, n1 * LANE)
                    acc_s[:, cs] = _dot(st['ob'], wo_v[:, cs]) + acc_s[:, cs]
                return fn

            def qp_slice(t):
                def fn():
                    g, n = divmod(t, GD // LANE)
                    cs = slice(n * LANE, (n + 1) * LANE)
                    q = _dot(st['h'], wq_v[:, :, t * LANE:(t + 1) * LANE].reshape(D, LANE))
                    q_s[g, :, cs] = jnp.where(diag[:, cs], q, 0.0).astype(BF16)
                return fn

            def mod_slice(t):
                def fn():
                    st.setdefault('mod', {})[t] = _dot(st['sc'], wm_v[:, :, t * LANE:(t + 1) * LANE].reshape(D, LANE))
                return fn

            def mod_part(i):
                return jnp.concatenate([st['mod'][t] for t in range(i * NS, (i + 1) * NS)], axis=1)

            def prep():
                c = c_v[...].astype(F32)
                sc = c * (1.0 / (1.0 + jnp.exp(-c)))
                st['sc'] = jnp.broadcast_to(sc, (M, D)).astype(BF16)
                x = x_v[...].reshape(1, D).astype(F32)
                st['x'] = jnp.broadcast_to(x, (M, D))
                st['lnx'] = _layernorm(st['x'])
                acc_s[...] = jnp.zeros((M, D), F32)

            def make_h():
                st['h'] = (st['lnx'] * (1.0 + mod_part(1)) + mod_part(0)).astype(BF16)

            hm = [streams(wm_hbm, wm_v, r, c, 768, S_V) for r in range(0, LANE, 8) for c in range(0, 6 * D, 768)]
            hq = [streams(wq_hbm, wq_v, r, c, 1024, S_V + 1) for r in range(0, LANE, 8) for c in range(0, H * DH, 1024)]
            head = hm + hq
            seq = head + [k_piece(0, j) for j in range(NT)]
            cp_c().start(priority=HI)
            cp_x().start(priority=HI)
            for mk in seq[:LA]:
                mk().start(priority=LO)
            work = {4: [prep]}
            for i, t0 in enumerate(range(0, 6 * NS, MOD[0])):
                work[len(hm) + MOD[1] * i] = [mod_slice(t) for t in range(t0, t0 + MOD[0])]
            work[max(work) + 1] = [make_h]
            phase([[mk] for mk in head], _spread(seq[LA:], len(head)),
                  _spread([rect(wg_hbm, wg_v, r, 8, c, F // 2, S_OTH) for r in range(0, D, 8) for c in (0, F // 2)],
                          len(head)),
                  work, {4: [lambda: cp_c().wait(), lambda: cp_x().wait()]})

            nq = H * DH // LANE
            work = {QP[1] * i: [qp_slice(t) for t in range(t0, min(nq, t0 + QP[0]))]
                    for i, t0 in enumerate(range(0, nq, QP[0]))}
            assert max(work) < NT
            small = [[mk] for mk in u_pieces(0) + d_pieces(0, WD0)]
            small += [[] for _ in range(CARVE0 - len(small))] + [v_small(0, j) for j in range(CARVE0, NT)]
            phase([[k_piece(0, j)] for j in range(NT)], [[v_bulk(0, j)] for j in range(NT)], small, work)

            def body(g, carry):
                small = [[mk] for mk in o_pieces(g) + u_pieces(g + 1)] + [v_small(g + 1, j) for j in range(CARVE0, NT)]
                work = {}
                j = 0
                for t in range(0, NT, QK[0]):
                    work[j] = [qk_slice(g, t, min(NT, t + QK[0]))]
                    j += QK[1]
                j -= QK[1] - 1
                work[j] = [max_fin]
                j += 1
                for t in range(0, NT, PV[0]):
                    t1 = min(NT, t + PV[0])
                    need = min(b for b in vbounds if b >= t1) - 1
                    j = max(j, need)
                    work[j] = [pv_slice(g, t, t1)]
                    j += PV[1]
                j -= PV[1] - 1
                work[j] = [pv_fin]
                jo = max(j + 2, NT + 14)
                work[jo] = [wo_slice(0, 3)]
                work[jo + 2] = [wo_slice(3, 5)]
                assert jo + 2 < 2 * NT
                phase([[v_bulk(g, j)] + v_small(g, j) for j in range(NT)], [[k_piece(g + 1, j)] for j in range(NT)],
                      small[:NT], work)
                phase([[k_piece(g + 1, j)] for j in range(NT)], [[v_bulk(g + 1, j)] for j in range(NT)],
                      small[NT:], {j - NT: w for j, w in work.items() if j >= NT}, {jo - NT: [wait_all(wo_v, S_O)]})
                return carry

            lax.fori_loop(0, NG - 1, body, 0)

            g = NG - 1
            work = {}
            t, j = 0, 0
            while t < NT:
                work[j] = [qk_slice(g, t, min(NT, t + LASTQK))]
                t += LASTQK
                j += 1
            work[j] = [max_fin]
            j += 1
            t = 0
            last = vbounds[-2]
            while t < last and j < NT:
                avail = max(b for b in vbounds if b <= j + 1)
                rem_ticks = NT - 2 - j
                n = 1 if (last - t) <= rem_ticks else 2
                n = min(n, avail - t)
                if n > 0:
                    work[j] = [pv_slice(g, t, t + n)]
                    t += n
                j += 1
            lastp = o_pieces(g) + d_pieces(WD0, WDF)
            small = _spread(lastp, NT) if WDF > WD0 else _spread(lastp, NT - 4) + [[]] * 4
            phase([[v_bulk(g, j)] + v_small(g, j) for j in range(NT)], [[cp_da, cp_db]] + [[]] * (NT - 1), small, work)

            if compute and not notail:
                pv_slice(g, t, NT)()
                pv_fin()
            wait_all(wo_v, S_O)()
            if compute and not notail:
                acc = _dot(st['ob'], wo_v[...]) + acc_s[...]
                attn = jnp.sum(acc, axis=0, keepdims=True)
                x1 = st['x'] + mod_part(2) * attn
                h2 = (_layernorm(x1) * (1.0 + mod_part(4)) + mod_part(3)).astype(BF16)
            wait_all(wg_v, S_OTH)()
            wait_all(wu_v, S_OTH)()
            if WDF:
                wait_all(wd_v.at[pl.ds(0, WDF), :], S_OTH)()
            if not compute or notail:
                cp_da().wait(); cp_db().wait()
                if notail:
                    r = (acc_s[...] + mod_part(2) + mod_part(3) + mod_part(4) + mod_part(5) + st['m'] + st['o'][:, 0:1] + st['l'][:, 0:1])[0:1]
                    o_ref[...] = r.reshape(1, 1, D).astype(o_ref.dtype)
                else:
                    o_ref[...] = x_v[...]
                return
            gg = _dot(h2, wg_v[...])
            uu = _dot(h2, wu_v[...])
            hh = (gg * uu).astype(BF16)
            cp_da().wait()
            ffn = _dot(hh[:, :F - WDB], wd_v[0:F - WDB, :])
            cp_db().wait()
            ffn = _dot(hh[:, F - WDB:], wd_v[F - WDB:F, :]) + ffn
            out = x1 + mod_part(5) * ffn
            if debug:
                o_ref[0] = out[0:1]
                o_ref[1] = attn
                o_ref[2] = ffn[0:1]
            else:
                o_ref[...] = out[0:1].reshape(1, 1, D).astype(o_ref.dtype)
        return kernel

    @jax.jit
    def fn(A_x, A_k_cache, A_v_cache, A_wq, A_wo, B_x, B_w_gate, B_w_up, B_w_down, c, w_mod):
        Sk = A_k_cache.shape[2]
        W = min(4096, max(256, Sk // 4))
        kt = jnp.swapaxes(A_k_cache, 2, 3).reshape(H * DH, Sk)
        vt = jnp.swapaxes(A_v_cache, 2, 3).reshape(H * DH, Sk)
        any_spec = pl.BlockSpec(memory_space=pl.ANY)
        out_shape = jax.ShapeDtypeStruct((3, 1, D), F32) if debug else jax.ShapeDtypeStruct((1, 1, D), A_x.dtype)
        return pl.pallas_call(
            make(Sk, W),
            out_shape=out_shape,
            in_specs=[any_spec] * 10,
            scratch_shapes=[
                pltpu.VMEM((1, 1, D), BF16),
                pltpu.VMEM((1, D), BF16),
                pltpu.VMEM((NS, LANE, 6 * D), BF16),
                pltpu.VMEM((NS, LANE, H * DH), BF16),
                pltpu.VMEM((GD, D), BF16),
                pltpu.VMEM((D, F), BF16),
                pltpu.VMEM((D, F), BF16),
                pltpu.VMEM((F, D), BF16),
                pltpu.VMEM((2, GD, W), BF16),
                pltpu.VMEM((2, GD, W), BF16),
                pltpu.VMEM((NG, M, GD), BF16),
                pltpu.VMEM((M, D), F32),
                pltpu.VMEM((M, W), F32),
                pltpu.SemaphoreType.DMA((NSEM,)),
            ],
            compiler_params=pltpu.CompilerParams(vmem_limit_bytes=64 * 1024 * 1024,
                                                 disable_bounds_checks=not checks,
                                                 disable_semaphore_checks=not checks),
        )(A_x, c, kt, vt, A_wq.reshape(NS, LANE, H * DH), A_wo, B_w_gate, B_w_up, B_w_down,
          w_mod.reshape(NS, LANE, 6 * D))
    return fn


_impl = build()


@jax.jit
def pallas_adaLN_cond__sliding_block_cached__glu_gated_bilinear__decode_kernel(
    A_x: jax.Array,
    A_k_cache: jax.Array,
    A_v_cache: jax.Array,
    A_wq: jax.Array,
    A_wo: jax.Array,
    B_x: jax.Array,
    B_w_gate: jax.Array,
    B_w_up: jax.Array,
    B_w_down: jax.Array,
    c: jax.Array,
    w_mod: jax.Array,
):
    return _impl(A_x, A_k_cache, A_v_cache, A_wq, A_wo, B_x, B_w_gate, B_w_up, B_w_down, c, w_mod)
```

```python
import jax
import jax.numpy as jnp
from jax import lax
import jax.experimental.pallas as pl
import jax.experimental.pallas.tpu as pltpu

F32 = jnp.float32
BF16 = jnp.bfloat16

D, H, DH, F = 640, 32, 192, 1536
G = 2
GD = G * DH
NG = H // G
M = 8
LANE = 128
NS = D // LANE
NT = 32
HI, LO = 0, 1
AHEAD = 32
CR, CARVE0 = 48, 18
VB = (0, 12, 24, NT)
WD_EARLY = 64
WD_MXU = ((WD_EARLY, 1152), (1152, 1408))
WD_VPU = ((1408, 1504), (1504, F))

S_K, S_O, S_FFN, S_A, S_B, S_C, S_V = range(7)
NSEM = S_V + 3


def _layernorm(x, eps=1e-5):
    m = jnp.mean(x, axis=-1, keepdims=True)
    xc = x - m
    v = jnp.mean(xc * xc, axis=-1, keepdims=True)
    return xc * lax.rsqrt(v + eps)


def _dot(a, b):
    return jnp.dot(a, b, preferred_element_type=F32)


def _dot_nt(a, b):
    return lax.dot_general(a, b, (((1,), (1,)), ((), ())), preferred_element_type=F32)


def _spread(items, n):
    out = [[] for _ in range(n)]
    for i, it in enumerate(items):
        out[i * n // len(items)].append(it)
    return out


def _tiles(t0, t1):
    return slice(t0 * LANE, t1 * LANE)


def _make_kernel(w0):
    scale = DH ** -0.5

    def kernel(x_hbm, c_hbm, k_hbm, v_hbm, wq_hbm, wo_hbm, wg_hbm, wu_hbm, wd_hbm, wm_hbm,
               o_ref,
               x_v, c_v, wm_v, wq_v, wo_v, wg_v, wu_v, wd_v, kbuf, vbuf, q_s, acc_s, s_s, sem):

        def copy(src, dst, s):
            return pltpu.make_async_copy(src, dst, sem.at[s])

        def wait_total(dst, s):
            copy(dst, dst, s).wait()

        def row0(g, mult, off):
            r = g * mult + off
            return r if isinstance(r, int) else pl.multiple_of(r, 8)

        def k_piece(g, j):
            return lambda: copy(k_hbm.at[pl.ds(row0(g, GD, 0), GD), pl.ds(w0 + j * LANE, LANE)],
                                kbuf.at[g % 2, :, pl.ds(j * LANE, LANE)], S_K)

        def v_rows(g, j, r, nr):
            s = S_V + sum(j >= b for b in VB[1:-1])
            return lambda: copy(v_hbm.at[pl.ds(row0(g, GD, r), nr), pl.ds(w0 + j * LANE, LANE)],
                                vbuf.at[g % 2, pl.ds(r, nr), pl.ds(j * LANE, LANE)], s)

        def v_bulk(g, j):
            return v_rows(g, j, 0, GD - CR if j >= CARVE0 else GD)

        def v_small(g, j):
            return [v_rows(g, j, GD - CR, CR)] if j >= CARVE0 else []

        def streams(src, dst, r, c, nc, s):
            return lambda: copy(src.at[:, pl.ds(r, 8), pl.ds(c, nc)], dst.at[:, pl.ds(r, 8), pl.ds(c, nc)], s)

        def rect(src, dst, r, nr, c, nc, s):
            return lambda: copy(src.at[pl.ds(r, nr), pl.ds(c, nc)], dst.at[pl.ds(r, nr), pl.ds(c, nc)], s)

        def wo_pieces(g):
            boxes = [b for r in range(0, GD, 48)
                     for b in ((r, 16, 0, 384), (r, 24, 384, 256), (r + 16, 16, 0, 384), (r + 32, 16, 0, 384),
                               (r + 24, 24, 384, 256))]
            return [(lambda r=r, nr=nr, c=c, nc=nc: copy(wo_hbm.at[pl.ds(row0(g, GD, r), nr), pl.ds(c, nc)],
                                                         wo_v.at[pl.ds(r, nr), pl.ds(c, nc)], S_O))
                    for r, nr, c, nc in boxes]

        def wu_pieces(n):
            return [rect(wu_hbm, wu_v, row0(n, D // NG, r), 8, c, F // 2, S_FFN)
                    for r in range(0, D // NG, 8) for c in (0, F // 2)]

        def cp_c():
            return copy(c_hbm, c_v, S_A)

        def cp_x():
            return copy(x_hbm, x_v, S_B)

        wd_last = [rect(wd_hbm, wd_v, r0, r1 - r0, 0, D, s)
                   for (r0, r1), s in zip(WD_MXU + WD_VPU, (S_A, S_B, S_K, S_C))]

        def phase(waits, bulk, small, work):
            for j in range(len(waits)):
                for mk in waits[j]:
                    mk().wait()
                for mk in bulk[j]:
                    mk().start(priority=LO)
                for mk in small[j]:
                    mk().start(priority=HI)
                for fn in work.get(j, ()):
                    fn()

        row = lax.broadcasted_iota(jnp.int32, (M, GD), 0)
        col = lax.broadcasted_iota(jnp.int32, (M, GD), 1)
        diag = (col >= row * DH) & (col < (row + 1) * DH)
        st = {'mod': {}}

        def prep():
            cp_c().wait()
            cp_x().wait()
            c = c_v[...].astype(F32)
            silu = c * (1.0 / (1.0 + jnp.exp(-c)))
            st['silu'] = jnp.broadcast_to(silu, (M, D)).astype(BF16)
            st['x'] = jnp.broadcast_to(x_v[...].reshape(1, D).astype(F32), (M, D))
            st['lnx'] = _layernorm(st['x'])
            acc_s[...] = jnp.zeros((M, D), F32)

        def mod_slice(t):
            def fn():
                st['mod'][t] = _dot(st['silu'], wm_v[:, :, _tiles(t, t + 1)].reshape(D, LANE))
            return fn

        def mod(i):
            return jnp.concatenate([st['mod'][t] for t in range(i * NS, (i + 1) * NS)], axis=1)

        def make_h():
            st['h'] = (st['lnx'] * (1.0 + mod(1)) + mod(0)).astype(BF16)

        def q_group(g):
            def fn():
                q = _dot(st['h'], wq_v[:, :, g * GD:(g + 1) * GD].reshape(D, GD))
                q_s[g] = jnp.where(diag, q, 0.0).astype(BF16)
            return fn

        def qk_slice(g, t0, t1):
            def fn():
                s = _dot(q_s[g], kbuf[g % 2, :, _tiles(t0, t1)])
                s_s[:, _tiles(t0, t1)] = s
                mx = s[:, _tiles(0, 1)]
                for u in range(1, t1 - t0):
                    mx = jnp.maximum(mx, s[:, _tiles(u, u + 1)])
                st['mx'] = mx if t0 == 0 else jnp.maximum(st['mx'], mx)
            return fn

        def row_max():
            st['m'] = jnp.max(st['mx'], axis=-1, keepdims=True)

        def pv_slice(g, t0, t1):
            def fn():
                p = jnp.exp((s_s[:, _tiles(t0, t1)] - st['m']) * scale)
                ps = p[:, _tiles(0, 1)]
                for u in range(1, t1 - t0):
                    ps = ps + p[:, _tiles(u, u + 1)]
                o = _dot_nt(p.astype(BF16), vbuf[g % 2, :, _tiles(t0, t1)])
                st['l'] = ps if t0 == 0 else st['l'] + ps
                st['o'] = o if t0 == 0 else o + st['o']
            return fn

        def normalize():
            l = jnp.sum(st['l'], axis=-1, keepdims=True)
            st['ob'] = jnp.where(diag, st['o'] / l, 0.0).astype(BF16)

        def wo_slice(t0, t1):
            def fn():
                acc_s[:, _tiles(t0, t1)] = _dot(st['ob'], wo_v[:, _tiles(t0, t1)]) + acc_s[:, _tiles(t0, t1)]
            return fn

        hm = [streams(wm_hbm, wm_v, r, c, 768, S_V) for r in range(0, LANE, 8) for c in range(0, 6 * D, 768)]
        hq = [streams(wq_hbm, wq_v, r, c, 1024, S_V + 1) for r in range(0, LANE, 8) for c in range(0, H * DH, 1024)]
        head = hm + hq
        bulk = head + [k_piece(0, j) for j in range(NT)]
        cp_c().start(priority=HI)
        cp_x().start(priority=HI)
        for mk in bulk[:AHEAD]:
            mk().start(priority=LO)
        work = {4: [prep]}
        for i in range(3 * NS):
            work[len(hm) + 5 * i] = [mod_slice(2 * i), mod_slice(2 * i + 1)]
        work[max(work) + 1] = [make_h]
        wg_pieces = [rect(wg_hbm, wg_v, r, 8, c, F // 2, S_FFN) for r in range(0, D, 8) for c in (0, F // 2)]
        phase([[mk] for mk in head], [[mk] for mk in bulk[AHEAD:]], _spread(wg_pieces, len(head)), work)

        small = wu_pieces(0) + [rect(wd_hbm, wd_v, r, 8, 0, D, S_FFN) for r in range(0, WD_EARLY, 8)]
        assert len(small) == CARVE0
        phase([[k_piece(0, j)] for j in range(NT)], [[v_bulk(0, j)] for j in range(NT)],
              [[mk] for mk in small] + [v_small(0, j) for j in range(CARVE0, NT)],
              {2 * g: [q_group(g)] for g in range(NG)})

        def body(g, carry):
            small = [[mk] for mk in wo_pieces(g) + wu_pieces(g + 1)]
            small += [v_small(g + 1, j) for j in range(CARVE0, NT)]
            work = {2 * i: [qk_slice(g, 4 * i, 4 * i + 4)] for i in range(8)}
            work[15] = [row_max]
            for i in range(16):
                work[16 + 2 * i] = [pv_slice(g, 2 * i, 2 * i + 2)]
            work[47] = [normalize]
            work[49] = [lambda: wait_total(wo_v, S_O), wo_slice(0, 3)]
            work[51] = [wo_slice(3, NS)]
            phase([[v_bulk(g, j)] + v_small(g, j) for j in range(NT)] + [[k_piece(g + 1, j)] for j in range(NT)],
                  [[k_piece(g + 1, j)] for j in range(NT)] + [[v_bulk(g + 1, j)] for j in range(NT)],
                  small, work)
            return carry

        lax.fori_loop(0, NG - 1, body, 0)

        g = NG - 1
        work = {j: [qk_slice(g, 3 * j, min(NT, 3 * j + 3))] for j in range(11)}
        work[11] = [row_max]
        for i in range(6):
            work[12 + i] = [pv_slice(g, 2 * i, 2 * i + 2)]
        for i in range(5):
            work[23 + i] = [pv_slice(g, 12 + 2 * i, 14 + 2 * i)]
        work[28] = [pv_slice(g, 22, 23)]
        work[29] = [pv_slice(g, 23, 24)]
        phase([[v_bulk(g, j)] + v_small(g, j) for j in range(NT)], [wd_last] + [[]] * (NT - 1),
              _spread(wo_pieces(g), NT - 4) + [[]] * 4, work)
        pv_slice(g, VB[2], NT)()
        normalize()

        wait_total(wo_v, S_O)
        attn = jnp.sum(_dot(st['ob'], wo_v[...]) + acc_s[...], axis=0, keepdims=True)
        x1 = st['x'] + mod(2) * attn
        h2 = (_layernorm(x1) * (1.0 + mod(4)) + mod(3)).astype(BF16)

        wait_total(wg_v, S_FFN)
        wait_total(wu_v, S_FFN)
        wait_total(wd_v.at[pl.ds(0, WD_EARLY), :], S_FFN)
        hh = (_dot(h2, wg_v[...]) * _dot(h2, wu_v[...])).astype(BF16)
        v0 = WD_VPU[0][0]
        hcol = jnp.broadcast_to(hh[0:1, v0:].astype(F32), (LANE, LANE)).T

        wd_last[0]().wait()
        r1 = WD_MXU[0][1]
        ffn = _dot(hh[:, :r1], wd_v[0:r1, :])
        wd_last[1]().wait()
        ffn = _dot(hh[:, r1:v0], wd_v[r1:v0, :]) + ffn
        part = None
        for mk, (a, b) in zip(wd_last[2:], WD_VPU):
            mk().wait()
            cols = [(wd_v[a:b, _tiles(t, t + 1)].astype(F32) * hcol[a - v0:b - v0])
                    .reshape((b - a) // 8, 8, LANE).sum(axis=0) for t in range(NS)]
            p8 = jnp.concatenate(cols, axis=1)
            part = p8 if part is None else part + p8
        ffn = ffn + jnp.sum(part, axis=0, keepdims=True)
        out = x1 + mod(5) * ffn
        o_ref[...] = out[0:1].reshape(1, 1, D).astype(o_ref.dtype)

    return kernel


@jax.jit
def pallas_adaLN_cond__sliding_block_cached__glu_gated_bilinear__decode_kernel(
    A_x: jax.Array,
    A_k_cache: jax.Array,
    A_v_cache: jax.Array,
    A_wq: jax.Array,
    A_wo: jax.Array,
    B_x: jax.Array,
    B_w_gate: jax.Array,
    B_w_up: jax.Array,
    B_w_down: jax.Array,
    c: jax.Array,
    w_mod: jax.Array,
):
    del B_x
    sk = A_k_cache.shape[2]
    w = min(4096, max(256, sk // 4))
    assert A_x.shape == (1, 1, D) and A_k_cache.shape == A_v_cache.shape == (1, H, sk, DH)
    assert w == NT * LANE and (sk - w) % LANE == 0
    kt = jnp.swapaxes(A_k_cache, 2, 3).reshape(H * DH, sk)
    vt = jnp.swapaxes(A_v_cache, 2, 3).reshape(H * DH, sk)
    return pl.pallas_call(
        _make_kernel(sk - w),
        out_shape=jax.ShapeDtypeStruct((1, 1, D), A_x.dtype),
        in_specs=[pl.BlockSpec(memory_space=pl.ANY)] * 10,
        scratch_shapes=[
            pltpu.VMEM((1, 1, D), BF16),
            pltpu.VMEM((1, D), BF16),
            pltpu.VMEM((NS, LANE, 6 * D), BF16),
            pltpu.VMEM((NS, LANE, H * DH), BF16),
            pltpu.VMEM((GD, D), BF16),
            pltpu.VMEM((D, F), BF16),
            pltpu.VMEM((D, F), BF16),
            pltpu.VMEM((F, D), BF16),
            pltpu.VMEM((2, GD, w), BF16),
            pltpu.VMEM((2, GD, w), BF16),
            pltpu.VMEM((NG, M, GD), BF16),
            pltpu.VMEM((M, D), F32),
            pltpu.VMEM((M, w), F32),
            pltpu.SemaphoreType.DMA((NSEM,)),
        ],
        compiler_params=pltpu.CompilerParams(
            vmem_limit_bytes=64 * 1024 * 1024,
            disable_bounds_checks=True,
            disable_semaphore_checks=True,
        ),
    )(A_x, c, kt, vt, A_wq.reshape(NS, LANE, H * DH), A_wo, B_w_gate, B_w_up, B_w_down,
      w_mod.reshape(NS, LANE, 6 * D))
```

```python
import jax
import jax.numpy as jnp
from jax import lax
import jax.experimental.pallas as pl
import jax.experimental.pallas.tpu as pltpu

F32 = jnp.float32
BF16 = jnp.bfloat16

D, H, DH, F = 640, 32, 192, 1536
G = 2
GD = G * DH
NG = H // G
M = 8
LANE = 128
NS = D // LANE
NT = 32
HI, LO = 0, 1
AHEAD = 32
CR, CARVE0 = 48, 18
PRE, CARVE_K0 = 8, 8
VB = (0, 12, 24, NT)
WD_EARLY = 64
WD_MXU = ((WD_EARLY, 1152), (1152, 1408))
WD_VPU = ((1408, 1504), (1504, F))

S_K, S_O, S_FFN, S_A, S_B, S_C, S_V = range(7)
NSEM = S_V + 3


def _layernorm(x, eps=1e-5):
    m = jnp.mean(x, axis=-1, keepdims=True)
    xc = x - m
    v = jnp.mean(xc * xc, axis=-1, keepdims=True)
    return xc * lax.rsqrt(v + eps)


def _dot(a, b):
    return jnp.dot(a, b, preferred_element_type=F32)


def _dot_nt(a, b):
    return lax.dot_general(a, b, (((1,), (1,)), ((), ())), preferred_element_type=F32)


def _spread(items, n):
    out = [[] for _ in range(n)]
    for i, it in enumerate(items):
        out[i * n // len(items)].append(it)
    return out


def _tiles(t0, t1):
    return slice(t0 * LANE, t1 * LANE)


def _make_kernel(w0):
    scale = DH ** -0.5

    def kernel(x_hbm, c_hbm, k_hbm, v_hbm, wq_hbm, wo_hbm, wg_hbm, wu_hbm, wd_hbm, wm_hbm,
               o_ref,
               x_v, c_v, wm_v, wq_v, wo_v, wg_v, wu_v, wd_v, kbuf, vbuf, q_s, acc_s, s_s, sem):

        def copy(src, dst, s):
            return pltpu.make_async_copy(src, dst, sem.at[s])

        def wait_total(dst, s):
            copy(dst, dst, s).wait()

        def row0(g, mult, off):
            r = g * mult + off
            return r if isinstance(r, int) else pl.multiple_of(r, 8)

        def k_piece(g, j, r=0, nr=GD):
            return lambda: copy(k_hbm.at[pl.ds(row0(g, GD, r), nr), pl.ds(w0 + j * LANE, LANE)],
                                kbuf.at[g % 2, pl.ds(r, nr), pl.ds(j * LANE, LANE)], S_K)

        def v_rows(g, j, r, nr):
            s = S_V + sum(j >= b for b in VB[1:-1])
            return lambda: copy(v_hbm.at[pl.ds(row0(g, GD, r), nr), pl.ds(w0 + j * LANE, LANE)],
                                vbuf.at[g % 2, pl.ds(r, nr), pl.ds(j * LANE, LANE)], s)

        def v_bulk(g, j):
            return v_rows(g, j, 0, GD - CR if j >= CARVE0 else GD)

        def v_small(g, j):
            return [v_rows(g, j, GD - CR, CR)] if j >= CARVE0 else []

        def streams(src, dst, r, c, nc, s):
            return lambda: copy(src.at[:, pl.ds(r, 8), pl.ds(c, nc)], dst.at[:, pl.ds(r, 8), pl.ds(c, nc)], s)

        def rect(src, dst, r, nr, c, nc, s):
            return lambda: copy(src.at[pl.ds(r, nr), pl.ds(c, nc)], dst.at[pl.ds(r, nr), pl.ds(c, nc)], s)

        def wo_pieces(g):
            boxes = [b for r in range(0, GD, 48)
                     for b in ((r, 16, 0, 384), (r, 24, 384, 256), (r + 16, 16, 0, 384), (r + 32, 16, 0, 384),
                               (r + 24, 24, 384, 256))]
            return [(lambda r=r, nr=nr, c=c, nc=nc: copy(wo_hbm.at[pl.ds(row0(g, GD, r), nr), pl.ds(c, nc)],
                                                         wo_v.at[pl.ds(r, nr), pl.ds(c, nc)], S_O))
                    for r, nr, c, nc in boxes]

        def wu_pieces(n):
            return [rect(wu_hbm, wu_v, row0(n, D // NG, r), 8, c, F // 2, S_FFN)
                    for r in range(0, D // NG, 8) for c in (0, F // 2)]

        def cp_c():
            return copy(c_hbm, c_v, S_A)

        def cp_x():
            return copy(x_hbm, x_v, S_B)

        wd_last = [rect(wd_hbm, wd_v, r0, r1 - r0, 0, D, s)
                   for (r0, r1), s in zip(WD_MXU + WD_VPU, (S_A, S_B, S_K, S_C))]

        def phase(waits, bulk, small, work):
            for j in range(len(waits)):
                for mk in waits[j]:
                    mk().wait()
                for mk in bulk[j]:
                    mk().start(priority=LO)
                for mk in small[j]:
                    mk().start(priority=HI)
                for fn in work.get(j, ()):
                    fn()

        row = lax.broadcasted_iota(jnp.int32, (M, GD), 0)
        col = lax.broadcasted_iota(jnp.int32, (M, GD), 1)
        diag = (col >= row * DH) & (col < (row + 1) * DH)
        st = {'mod': {}}

        def prep():
            cp_c().wait()
            cp_x().wait()
            c = c_v[...].astype(F32)
            silu = c * (1.0 / (1.0 + jnp.exp(-c)))
            st['silu'] = jnp.broadcast_to(silu, (M, D)).astype(BF16)
            st['x'] = jnp.broadcast_to(x_v[...].reshape(1, D).astype(F32), (M, D))
            st['lnx'] = _layernorm(st['x'])
            acc_s[...] = jnp.zeros((M, D), F32)

        def mod_slice(t):
            def fn():
                st['mod'][t] = _dot(st['silu'], wm_v[:, :, _tiles(t, t + 1)].reshape(D, LANE))
            return fn

        def mod(i):
            return jnp.concatenate([st['mod'][t] for t in range(i * NS, (i + 1) * NS)], axis=1)

        def make_h():
            st['h'] = (st['lnx'] * (1.0 + mod(1)) + mod(0)).astype(BF16)

        def q_group(g):
            def fn():
                q = _dot(st['h'], wq_v[:, :, g * GD:(g + 1) * GD].reshape(D, GD))
                q_s[g] = jnp.where(diag, q, 0.0).astype(BF16)
            return fn

        def qk_slice(g, t0, t1):
            def fn():
                s = _dot(q_s[g], kbuf[g % 2, :, _tiles(t0, t1)])
                s_s[:, _tiles(t0, t1)] = s
                mx = s[:, _tiles(0, 1)]
                for u in range(1, t1 - t0):
                    mx = jnp.maximum(mx, s[:, _tiles(u, u + 1)])
                st['mx'] = mx if t0 == 0 else jnp.maximum(st['mx'], mx)
            return fn

        def row_max():
            st['m'] = jnp.max(st['mx'], axis=-1, keepdims=True)

        def pv_slice(g, t0, t1):
            def fn():
                p = jnp.exp((s_s[:, _tiles(t0, t1)] - st['m']) * scale)
                ps = p[:, _tiles(0, 1)]
                for u in range(1, t1 - t0):
                    ps = ps + p[:, _tiles(u, u + 1)]
                o = _dot_nt(p.astype(BF16), vbuf[g % 2, :, _tiles(t0, t1)])
                st['l'] = ps if t0 == 0 else st['l'] + ps
                st['o'] = o if t0 == 0 else o + st['o']
            return fn

        def normalize():
            l = jnp.sum(st['l'], axis=-1, keepdims=True)
            st['ob'] = jnp.where(diag, st['o'] / l, 0.0).astype(BF16)

        def wo_slice(t0, t1):
            def fn():
                acc_s[:, _tiles(t0, t1)] = _dot(st['ob'], wo_v[:, _tiles(t0, t1)]) + acc_s[:, _tiles(t0, t1)]
            return fn

        hm = [streams(wm_hbm, wm_v, r, c, 768, S_V) for r in range(0, LANE, 8) for c in range(0, 6 * D, 768)]
        hq = [streams(wq_hbm, wq_v, r, c, 1024, S_V + 1) for r in range(0, LANE, 8) for c in range(0, H * DH, 1024)]
        head = hm + hq
        k0_bulk = [k_piece(0, j, 0, GD - CR if j >= CARVE_K0 else GD) for j in range(NT)]
        k0_small = [[k_piece(0, j, GD - CR, CR)] if j >= CARVE_K0 else [] for j in range(NT)]
        bulk = head + k0_bulk
        wg_pieces = [rect(wg_hbm, wg_v, r, 8, c, F // 2, S_FFN) for r in range(0, D, 8) for c in (0, F // 2)]
        cp_c().start(priority=HI)
        cp_x().start(priority=HI)
        for i, mk in enumerate(bulk[:AHEAD]):
            mk().start(priority=LO)
            if i % (AHEAD // PRE) == AHEAD // PRE - 1:
                wg_pieces[i * PRE // AHEAD]().start(priority=HI)
        small = [[mk] for mk in wg_pieces[PRE:]] + k0_small[CARVE_K0:]
        assert len(small) == len(head) == len(bulk) - AHEAD
        work = {4: [prep]}
        for i in range(3 * NS):
            work[len(hm) + 5 * i] = [mod_slice(2 * i), mod_slice(2 * i + 1)]
        work[max(work) + 1] = [make_h]
        phase([[mk] for mk in head], [[mk] for mk in bulk[AHEAD:]], small, work)

        small = wu_pieces(0) + [rect(wd_hbm, wd_v, r, 8, 0, D, S_FFN) for r in range(0, WD_EARLY, 8)]
        assert len(small) == CARVE0
        phase([[k0_bulk[j]] + k0_small[j] for j in range(NT)], [[v_bulk(0, j)] for j in range(NT)],
              [[mk] for mk in small] + [v_small(0, j) for j in range(CARVE0, NT)],
              {2 * g: [q_group(g)] for g in range(NG)})

        def body(g, carry):
            small = [[mk] for mk in wo_pieces(g) + wu_pieces(g + 1)]
            small += [v_small(g + 1, j) for j in range(CARVE0, NT)]
            work = {2 * i: [qk_slice(g, 4 * i, 4 * i + 4)] for i in range(8)}
            work[15] = [row_max]
            for i in range(16):
                work[16 + 2 * i] = [pv_slice(g, 2 * i, 2 * i + 2)]
            work[47] = [normalize]
            work[49] = [lambda: wait_total(wo_v, S_O), wo_slice(0, 3)]
            work[51] = [wo_slice(3, NS)]
            phase([[v_bulk(g, j)] + v_small(g, j) for j in range(NT)] + [[k_piece(g + 1, j)] for j in range(NT)],
                  [[k_piece(g + 1, j)] for j in range(NT)] + [[v_bulk(g + 1, j)] for j in range(NT)],
                  small, work)
            return carry

        lax.fori_loop(0, NG - 1, body, 0)

        g = NG - 1
        work = {j: [qk_slice(g, 3 * j, min(NT, 3 * j + 3))] for j in range(11)}
        work[11] = [row_max]
        for i in range(6):
            work[12 + i] = [pv_slice(g, 2 * i, 2 * i + 2)]
        for i in range(5):
            work[23 + i] = [pv_slice(g, 12 + 2 * i, 14 + 2 * i)]
        work[28] = [pv_slice(g, 22, 23)]
        work[29] = [pv_slice(g, 23, 24)]
        phase([[v_bulk(g, j)] + v_small(g, j) for j in range(NT)], [wd_last] + [[]] * (NT - 1),
              _spread(wo_pieces(g), NT - 4) + [[]] * 4, work)
        pv_slice(g, VB[2], NT)()
        normalize()

        wait_total(wo_v, S_O)
        attn = jnp.sum(_dot(st['ob'], wo_v[...]) + acc_s[...], axis=0, keepdims=True)
        x1 = st['x'] + mod(2) * attn
        h2 = (_layernorm(x1) * (1.0 + mod(4)) + mod(3)).astype(BF16)

        wait_total(wg_v, S_FFN)
        wait_total(wu_v, S_FFN)
        wait_total(wd_v.at[pl.ds(0, WD_EARLY), :], S_FFN)
        hh = (_dot(h2, wg_v[...]) * _dot(h2, wu_v[...])).astype(BF16)
        v0 = WD_VPU[0][0]
        hcol = jnp.broadcast_to(hh[0:1, v0:].astype(F32), (LANE, LANE)).T

        wd_last[0]().wait()
        r1 = WD_MXU[0][1]
        ffn = _dot(hh[:, :r1], wd_v[0:r1, :])
        wd_last[1]().wait()
        ffn = _dot(hh[:, r1:v0], wd_v[r1:v0, :]) + ffn
        part = None
        for mk, (a, b) in zip(wd_last[2:], WD_VPU):
            mk().wait()
            cols = [(wd_v[a:b, _tiles(t, t + 1)].astype(F32) * hcol[a - v0:b - v0])
                    .reshape((b - a) // 8, 8, LANE).sum(axis=0) for t in range(NS)]
            p8 = jnp.concatenate(cols, axis=1)
            part = p8 if part is None else part + p8
        ffn = ffn + jnp.sum(part, axis=0, keepdims=True)
        out = x1 + mod(5) * ffn
        o_ref[...] = out[0:1].reshape(1, 1, D).astype(o_ref.dtype)

    return kernel


@jax.jit
def pallas_adaLN_cond__sliding_block_cached__glu_gated_bilinear__decode_kernel(
    A_x: jax.Array,
    A_k_cache: jax.Array,
    A_v_cache: jax.Array,
    A_wq: jax.Array,
    A_wo: jax.Array,
    B_x: jax.Array,
    B_w_gate: jax.Array,
    B_w_up: jax.Array,
    B_w_down: jax.Array,
    c: jax.Array,
    w_mod: jax.Array,
):
    del B_x
    sk = A_k_cache.shape[2]
    w = min(4096, max(256, sk // 4))
    assert A_x.shape == (1, 1, D) and A_k_cache.shape == A_v_cache.shape == (1, H, sk, DH)
    assert w == NT * LANE and (sk - w) % LANE == 0
    kt = jnp.swapaxes(A_k_cache, 2, 3).reshape(H * DH, sk)
    vt = jnp.swapaxes(A_v_cache, 2, 3).reshape(H * DH, sk)
    return pl.pallas_call(
        _make_kernel(sk - w),
        out_shape=jax.ShapeDtypeStruct((1, 1, D), A_x.dtype),
        in_specs=[pl.BlockSpec(memory_space=pl.ANY)] * 10,
        scratch_shapes=[
            pltpu.VMEM((1, 1, D), BF16),
            pltpu.VMEM((1, D), BF16),
            pltpu.VMEM((NS, LANE, 6 * D), BF16),
            pltpu.VMEM((NS, LANE, H * DH), BF16),
            pltpu.VMEM((GD, D), BF16),
            pltpu.VMEM((D, F), BF16),
            pltpu.VMEM((D, F), BF16),
            pltpu.VMEM((F, D), BF16),
            pltpu.VMEM((2, GD, w), BF16),
            pltpu.VMEM((2, GD, w), BF16),
            pltpu.VMEM((NG, M, GD), BF16),
            pltpu.VMEM((M, D), F32),
            pltpu.VMEM((M, w), F32),
            pltpu.SemaphoreType.DMA((NSEM,)),
        ],
        compiler_params=pltpu.CompilerParams(
            vmem_limit_bytes=64 * 1024 * 1024,
            disable_bounds_checks=True,
            disable_semaphore_checks=True,
        ),
    )(A_x, c, kt, vt, A_wq.reshape(NS, LANE, H * DH), A_wo, B_w_gate, B_w_up, B_w_down,
      w_mod.reshape(NS, LANE, 6 * D))
```

```python
import jax
import jax.numpy as jnp
from jax import lax
import jax.experimental.pallas as pl
import jax.experimental.pallas.tpu as pltpu

F32 = jnp.float32
BF16 = jnp.bfloat16

D, H, DH, F = 640, 32, 192, 1536
G = 2
GD = G * DH
NG = H // G
M = 8
LANE = 128
NS = D // LANE
NT = 32
HI, LO = 0, 1
AHEAD = 32
CR, CARVE0 = 48, 18
PRE, CARVE_K0 = 8, 8
VB = (0, 12, 24, NT)
WD_EARLY = 64
WD_MXU = ((WD_EARLY, 1152), (1152, 1408))
WD_VPU = ((1408, 1504), (1504, F))

S_K, S_O, S_FFN, S_A, S_B, S_C, S_V = range(7)
NSEM = S_V + 3


def _layernorm(x, eps=1e-5):
    m = jnp.mean(x, axis=-1, keepdims=True)
    xc = x - m
    v = jnp.mean(xc * xc, axis=-1, keepdims=True)
    return xc * lax.rsqrt(v + eps)


def _dot(a, b):
    return jnp.dot(a, b, preferred_element_type=F32)


def _dot_nt(a, b):
    return lax.dot_general(a, b, (((1,), (1,)), ((), ())), preferred_element_type=F32)


def _spread(items, n):
    out = [[] for _ in range(n)]
    for i, it in enumerate(items):
        out[i * n // len(items)].append(it)
    return out


def _tiles(t0, t1):
    return slice(t0 * LANE, t1 * LANE)


def _make_kernel(w0):
    scale = DH ** -0.5

    def kernel(x_hbm, c_hbm, k_hbm, v_hbm, wq_hbm, wo_hbm, wg_hbm, wu_hbm, wd_hbm, wm_hbm,
               o_ref,
               x_v, c_v, wm_v, wq_v, wo_v, wg_v, wu_v, wd_v, kbuf, vbuf, q_s, acc_s, s_s, sem):

        def copy(src, dst, s):
            return pltpu.make_async_copy(src, dst, sem.at[s])

        def wait_total(dst, s):
            copy(dst, dst, s).wait()

        def row0(g, mult, off):
            r = g * mult + off
            return r if isinstance(r, int) else pl.multiple_of(r, 8)

        def k_piece(g, j, r=0, nr=GD):
            return lambda: copy(k_hbm.at[pl.ds(row0(g, GD, r), nr), pl.ds(w0 + j * LANE, LANE)],
                                kbuf.at[g % 2, pl.ds(r, nr), pl.ds(j * LANE, LANE)], S_K)

        def v_rows(g, j, r, nr):
            s = S_V + sum(j >= b for b in VB[1:-1])
            return lambda: copy(v_hbm.at[pl.ds(row0(g, GD, r), nr), pl.ds(w0 + j * LANE, LANE)],
                                vbuf.at[g % 2, pl.ds(r, nr), pl.ds(j * LANE, LANE)], s)

        def v_bulk(g, j):
            return v_rows(g, j, 0, GD - CR if j >= CARVE0 else GD)

        def v_small(g, j):
            return [v_rows(g, j, GD - CR, CR)] if j >= CARVE0 else []

        def streams(src, dst, r, c, nc, s):
            return lambda: copy(src.at[:, pl.ds(r, 8), pl.ds(c, nc)], dst.at[:, pl.ds(r, 8), pl.ds(c, nc)], s)

        def rect(src, dst, r, nr, c, nc, s):
            return lambda: copy(src.at[pl.ds(r, nr), pl.ds(c, nc)], dst.at[pl.ds(r, nr), pl.ds(c, nc)], s)

        def wo_pieces(g):
            boxes = [b for r in range(0, GD, 48)
                     for b in ((r, 16, 0, 384), (r, 24, 384, 256), (r + 16, 16, 0, 384), (r + 32, 16, 0, 384),
                               (r + 24, 24, 384, 256))]
            return [(lambda r=r, nr=nr, c=c, nc=nc: copy(wo_hbm.at[pl.ds(row0(g, GD, r), nr), pl.ds(c, nc)],
                                                         wo_v.at[pl.ds(r, nr), pl.ds(c, nc)], S_O))
                    for r, nr, c, nc in boxes]

        def wu_pieces(n):
            return [rect(wu_hbm, wu_v, row0(n, D // NG, r), 8, c, F // 2, S_FFN)
                    for r in range(0, D // NG, 8) for c in (0, F // 2)]

        def cp_c():
            return copy(c_hbm, c_v, S_A)

        def cp_x():
            return copy(x_hbm, x_v, S_B)

        wd_last = [rect(wd_hbm, wd_v, r0, r1 - r0, 0, D, s)
                   for (r0, r1), s in zip(WD_MXU + WD_VPU, (S_A, S_B, S_K, S_C))]

        def phase(waits, bulk, small, work):
            for j in range(len(waits)):
                for mk in waits[j]:
                    mk().wait()
                for mk in bulk[j]:
                    mk().start(priority=LO)
                for mk in small[j]:
                    mk().start(priority=HI)
                for fn in work.get(j, ()):
                    fn()

        row = lax.broadcasted_iota(jnp.int32, (M, GD), 0)
        col = lax.broadcasted_iota(jnp.int32, (M, GD), 1)
        diag = (col >= row * DH) & (col < (row + 1) * DH)
        st = {'mod': {}}

        def prep():
            cp_c().wait()
            cp_x().wait()
            c = c_v[...].astype(F32)
            silu = c * (1.0 / (1.0 + jnp.exp(-c)))
            st['silu'] = jnp.broadcast_to(silu, (M, D)).astype(BF16)
            st['x'] = jnp.broadcast_to(x_v[...].reshape(1, D).astype(F32), (M, D))
            st['lnx'] = _layernorm(st['x'])
            acc_s[...] = jnp.zeros((M, D), F32)

        def mod_slice(t):
            def fn():
                st['mod'][t] = _dot(st['silu'], wm_v[:, :, _tiles(t, t + 1)].reshape(D, LANE))
            return fn

        def mod(i):
            return jnp.concatenate([st['mod'][t] for t in range(i * NS, (i + 1) * NS)], axis=1)

        def make_h():
            st['h'] = (st['lnx'] * (1.0 + mod(1)) + mod(0)).astype(BF16)

        def q_group(g):
            def fn():
                q = _dot(st['h'], wq_v[:, :, g * GD:(g + 1) * GD].reshape(D, GD))
                q_s[g] = jnp.where(diag, q, 0.0).astype(BF16)
            return fn

        def qk_slice(g, t0, t1):
            def fn():
                s = _dot(q_s[g], kbuf[g % 2, :, _tiles(t0, t1)])
                s_s[:, _tiles(t0, t1)] = s
                mx = s[:, _tiles(0, 1)]
                for u in range(1, t1 - t0):
                    mx = jnp.maximum(mx, s[:, _tiles(u, u + 1)])
                st['mx'] = mx if t0 == 0 else jnp.maximum(st['mx'], mx)
            return fn

        def row_max():
            st['m'] = jnp.max(st['mx'], axis=-1, keepdims=True)

        def pv_slice(g, t0, t1):
            def fn():
                p = jnp.exp((s_s[:, _tiles(t0, t1)] - st['m']) * scale)
                ps = p[:, _tiles(0, 1)]
                for u in range(1, t1 - t0):
                    ps = ps + p[:, _tiles(u, u + 1)]
                o = _dot_nt(p.astype(BF16), vbuf[g % 2, :, _tiles(t0, t1)])
                st['l'] = ps if t0 == 0 else st['l'] + ps
                st['o'] = o if t0 == 0 else o + st['o']
            return fn

        def normalize():
            l = jnp.sum(st['l'], axis=-1, keepdims=True)
            st['ob'] = jnp.where(diag, st['o'] / l, 0.0).astype(BF16)

        def wo_slice(t0, t1):
            def fn():
                acc_s[:, _tiles(t0, t1)] = _dot(st['ob'], wo_v[:, _tiles(t0, t1)]) + acc_s[:, _tiles(t0, t1)]
            return fn

        hm = [streams(wm_hbm, wm_v, r, c, 768, S_V) for r in range(0, LANE, 8) for c in range(0, 6 * D, 768)]
        hq = [streams(wq_hbm, wq_v, r, c, 1024, S_V + 1) for r in range(0, LANE, 8) for c in range(0, H * DH, 1024)]
        head = hm + hq
        k0_bulk = [k_piece(0, j, 0, GD - CR if j >= CARVE_K0 else GD) for j in range(NT)]
        k0_small = [[k_piece(0, j, GD - CR, CR)] if j >= CARVE_K0 else [] for j in range(NT)]
        bulk = head + k0_bulk
        wg_pieces = [rect(wg_hbm, wg_v, r, 8, c, F // 2, S_FFN) for r in range(0, D, 8) for c in (0, F // 2)]
        cp_c().start(priority=HI)
        cp_x().start(priority=HI)
        for i, mk in enumerate(bulk[:AHEAD]):
            mk().start(priority=LO)
            if i % (AHEAD // PRE) == AHEAD // PRE - 1:
                wg_pieces[i * PRE // AHEAD]().start(priority=HI)
        small = [[mk] for mk in wg_pieces[PRE:]] + k0_small[CARVE_K0:]
        assert len(small) == len(head) == len(bulk) - AHEAD
        work = {4: [prep]}
        for i in range(3 * NS):
            work[len(hm) + 5 * i] = [mod_slice(2 * i), mod_slice(2 * i + 1)]
        work[max(work) + 1] = [make_h]
        phase([[mk] for mk in head], [[mk] for mk in bulk[AHEAD:]], small, work)

        small = wu_pieces(0) + [rect(wd_hbm, wd_v, r, 8, 0, D, S_FFN) for r in range(0, WD_EARLY, 8)]
        assert len(small) == CARVE0
        phase([[k0_bulk[j]] + k0_small[j] for j in range(NT)], [[v_bulk(0, j)] for j in range(NT)],
              [[mk] for mk in small] + [v_small(0, j) for j in range(CARVE0, NT)],
              {2 * g: [q_group(g)] for g in range(NG)})

        def body(g, carry):
            small = [[mk] for mk in wo_pieces(g) + wu_pieces(g + 1)]
            small += [v_small(g + 1, j) for j in range(CARVE0, NT)]
            work = {2 * i: [qk_slice(g, 4 * i, 4 * i + 4)] for i in range(8)}
            work[15] = [row_max]
            for i in range(16):
                work[16 + 2 * i] = [pv_slice(g, 2 * i, 2 * i + 2)]
            work[47] = [normalize]
            work[49] = [lambda: wait_total(wo_v, S_O), wo_slice(0, 3)]
            work[51] = [wo_slice(3, NS)]
            phase([[v_bulk(g, j)] + v_small(g, j) for j in range(NT)] + [[k_piece(g + 1, j)] for j in range(NT)],
                  [[k_piece(g + 1, j)] for j in range(NT)] + [[v_bulk(g + 1, j)] for j in range(NT)],
                  small, work)
            return carry

        lax.fori_loop(0, NG - 1, body, 0)

        g = NG - 1
        work = {j: [qk_slice(g, 3 * j, min(NT, 3 * j + 3))] for j in range(11)}
        work[11] = [row_max]
        for i in range(6):
            work[12 + i] = [pv_slice(g, 2 * i, 2 * i + 2)]
        for i in range(5):
            work[23 + i] = [pv_slice(g, 12 + 2 * i, 14 + 2 * i)]
        work[28] = [pv_slice(g, 22, 23)]
        work[29] = [pv_slice(g, 23, 24)]
        phase([[v_bulk(g, j)] + v_small(g, j) for j in range(NT)], [wd_last] + [[]] * (NT - 1),
              _spread(wo_pieces(g), NT - 4) + [[]] * 4, work)
        pv_slice(g, VB[2], NT)()
        normalize()

        wait_total(wo_v, S_O)
        attn = jnp.sum(_dot(st['ob'], wo_v[...]) + acc_s[...], axis=0, keepdims=True)
        x1 = st['x'] + mod(2) * attn
        h2 = (_layernorm(x1) * (1.0 + mod(4)) + mod(3)).astype(BF16)

        wait_total(wg_v, S_FFN)
        wait_total(wu_v, S_FFN)
        wait_total(wd_v.at[pl.ds(0, WD_EARLY), :], S_FFN)
        hh = (_dot(h2, wg_v[...]) * _dot(h2, wu_v[...])).astype(BF16)
        v0 = WD_VPU[0][0]
        hcol = jnp.broadcast_to(hh[0:1, v0:].astype(F32), (LANE, LANE)).T

        wd_last[0]().wait()
        r1 = WD_MXU[0][1]
        ffn = _dot(hh[:, :r1], wd_v[0:r1, :])
        wd_last[1]().wait()
        ffn = _dot(hh[:, r1:v0], wd_v[r1:v0, :]) + ffn
        part = None
        for mk, (a, b) in zip(wd_last[2:], WD_VPU):
            mk().wait()
            cols = [(wd_v[a:b, _tiles(t, t + 1)].astype(F32) * hcol[a - v0:b - v0])
                    .reshape((b - a) // 8, 8, LANE).sum(axis=0) for t in range(NS)]
            p8 = jnp.concatenate(cols, axis=1)
            part = p8 if part is None else part + p8
        ffn = ffn + jnp.sum(part, axis=0, keepdims=True)
        out = x1 + mod(5) * ffn
        o_ref[...] = out[0:1].reshape(1, 1, D).astype(o_ref.dtype)

    return kernel


def _compiler_params():
    vmem = 64 * 1024 * 1024
    try:
        return pltpu.CompilerParams(vmem_limit_bytes=vmem, disable_bounds_checks=True,
                                    disable_semaphore_checks=True)
    except TypeError:
        return pltpu.CompilerParams(vmem_limit_bytes=vmem)


@jax.jit
def pallas_adaLN_cond__sliding_block_cached__glu_gated_bilinear__decode_kernel(
    A_x: jax.Array,
    A_k_cache: jax.Array,
    A_v_cache: jax.Array,
    A_wq: jax.Array,
    A_wo: jax.Array,
    B_x: jax.Array,
    B_w_gate: jax.Array,
    B_w_up: jax.Array,
    B_w_down: jax.Array,
    c: jax.Array,
    w_mod: jax.Array,
):
    del B_x
    sk = A_k_cache.shape[2]
    w = min(4096, max(256, sk // 4))
    assert A_x.shape == (1, 1, D) and A_k_cache.shape == A_v_cache.shape == (1, H, sk, DH)
    assert w == NT * LANE and (sk - w) % LANE == 0
    kt = jnp.swapaxes(A_k_cache, 2, 3).reshape(H * DH, sk)
    vt = jnp.swapaxes(A_v_cache, 2, 3).reshape(H * DH, sk)
    return pl.pallas_call(
        _make_kernel(sk - w),
        out_shape=jax.ShapeDtypeStruct((1, 1, D), A_x.dtype),
        in_specs=[pl.BlockSpec(memory_space=pl.ANY)] * 10,
        scratch_shapes=[
            pltpu.VMEM((1, 1, D), BF16),
            pltpu.VMEM((1, D), BF16),
            pltpu.VMEM((NS, LANE, 6 * D), BF16),
            pltpu.VMEM((NS, LANE, H * DH), BF16),
            pltpu.VMEM((GD, D), BF16),
            pltpu.VMEM((D, F), BF16),
            pltpu.VMEM((D, F), BF16),
            pltpu.VMEM((F, D), BF16),
            pltpu.VMEM((2, GD, w), BF16),
            pltpu.VMEM((2, GD, w), BF16),
            pltpu.VMEM((NG, M, GD), BF16),
            pltpu.VMEM((M, D), F32),
            pltpu.VMEM((M, w), F32),
            pltpu.SemaphoreType.DMA((NSEM,)),
        ],
        compiler_params=_compiler_params(),
    )(A_x, c, kt, vt, A_wq.reshape(NS, LANE, H * DH), A_wo, B_w_gate, B_w_up, B_w_down,
      w_mod.reshape(NS, LANE, 6 * D))
```

```python
import jax
import jax.numpy as jnp
from jax import lax
import jax.experimental.pallas as pl
import jax.experimental.pallas.tpu as pltpu

F32 = jnp.float32
BF16 = jnp.bfloat16

D, H, DH, F = 640, 32, 192, 1536
G = 2
GD = G * DH
NG = H // G
M = 8
LANE = 128
NS = D // LANE
NT = 32
HI, LO = 0, 1
AHEAD = 32
CR, CARVE0 = 48, 18
PRE, CARVE_K0 = 8, 8
VB = (0, 12, 24, NT)
WD_EARLY = 64
WD_MXU = ((WD_EARLY, 1152), (1152, 1408))
WD_VPU = ((1408, 1504), (1504, F))

S_K, S_O, S_G, S_U, S_D, S_A, S_B, S_C, S_V = range(9)
NSEM = S_V + 3


def _layernorm(x, eps=1e-5):
    m = jnp.mean(x, axis=-1, keepdims=True)
    xc = x - m
    v = jnp.mean(xc * xc, axis=-1, keepdims=True)
    return xc * lax.rsqrt(v + eps)


def _dot(a, b):
    return jnp.dot(a, b, preferred_element_type=F32)


def _dot_nt(a, b):
    return lax.dot_general(a, b, (((1,), (1,)), ((), ())), preferred_element_type=F32)


def _spread(items, n):
    out = [[] for _ in range(n)]
    for i, it in enumerate(items):
        out[i * n // len(items)].append(it)
    return out


def _tiles(t0, t1):
    return slice(t0 * LANE, t1 * LANE)


def _make_kernel(w0):
    scale = DH ** -0.5

    def kernel(x_hbm, c_hbm, k_hbm, v_hbm, wq_hbm, wo_hbm, wg_hbm, wu_hbm, wd_hbm, wm_hbm,
               o_ref,
               x_v, c_v, wm_v, wq_v, wo_v, wg_v, wu_v, wd_v, kbuf, vbuf, q_s, acc_s, s_s, sem):

        def copy(src, dst, s):
            return pltpu.make_async_copy(src, dst, sem.at[s])

        def wait_total(dst, s):
            copy(dst, dst, s).wait()

        def row0(g, mult, off):
            r = g * mult + off
            return r if isinstance(r, int) else pl.multiple_of(r, 8)

        def k_piece(g, j, r=0, nr=GD):
            return lambda: copy(k_hbm.at[pl.ds(row0(g, GD, r), nr), pl.ds(w0 + j * LANE, LANE)],
                                kbuf.at[g % 2, pl.ds(r, nr), pl.ds(j * LANE, LANE)], S_K)

        def v_rows(g, j, r, nr):
            s = S_V + sum(j >= b for b in VB[1:-1])
            return lambda: copy(v_hbm.at[pl.ds(row0(g, GD, r), nr), pl.ds(w0 + j * LANE, LANE)],
                                vbuf.at[g % 2, pl.ds(r, nr), pl.ds(j * LANE, LANE)], s)

        def v_bulk(g, j):
            return v_rows(g, j, 0, GD - CR if j >= CARVE0 else GD)

        def v_small(g, j):
            return [v_rows(g, j, GD - CR, CR)] if j >= CARVE0 else []

        def streams(src, dst, r, c, nc, s):
            return lambda: copy(src.at[:, pl.ds(r, 8), pl.ds(c, nc)], dst.at[:, pl.ds(r, 8), pl.ds(c, nc)], s)

        def rect(src, dst, r, nr, c, nc, s):
            return lambda: copy(src.at[pl.ds(r, nr), pl.ds(c, nc)], dst.at[pl.ds(r, nr), pl.ds(c, nc)], s)

        def wo_pieces(g):
            boxes = [b for r in range(0, GD, 48)
                     for b in ((r, 16, 0, 384), (r, 24, 384, 256), (r + 16, 16, 0, 384), (r + 32, 16, 0, 384),
                               (r + 24, 24, 384, 256))]
            return [(lambda r=r, nr=nr, c=c, nc=nc: copy(wo_hbm.at[pl.ds(row0(g, GD, r), nr), pl.ds(c, nc)],
                                                         wo_v.at[pl.ds(r, nr), pl.ds(c, nc)], S_O))
                    for r, nr, c, nc in boxes]

        def wu_pieces(n):
            return [rect(wu_hbm, wu_v, row0(n, D // NG, r), 8, c, F // 2, S_U)
                    for r in range(0, D // NG, 8) for c in (0, F // 2)]

        def cp_c():
            return copy(c_hbm, c_v, S_A)

        def cp_x():
            return copy(x_hbm, x_v, S_B)

        wd_last = [rect(wd_hbm, wd_v, r0, r1 - r0, 0, D, s)
                   for (r0, r1), s in zip(WD_MXU + WD_VPU, (S_A, S_B, S_K, S_C))]

        def phase(waits, bulk, small, work):
            for j in range(len(waits)):
                for mk in waits[j]:
                    mk().wait()
                for mk in bulk[j]:
                    mk().start(priority=LO)
                for mk in small[j]:
                    mk().start(priority=HI)
                for fn in work.get(j, ()):
                    fn()

        row = lax.broadcasted_iota(jnp.int32, (M, GD), 0)
        col = lax.broadcasted_iota(jnp.int32, (M, GD), 1)
        diag = (col >= row * DH) & (col < (row + 1) * DH)
        st = {'mod': {}}

        def prep():
            cp_c().wait()
            cp_x().wait()
            c = c_v[...].astype(F32)
            silu = c * (1.0 / (1.0 + jnp.exp(-c)))
            st['silu'] = jnp.broadcast_to(silu, (M, D)).astype(BF16)
            st['x'] = jnp.broadcast_to(x_v[...].reshape(1, D).astype(F32), (M, D))
            st['lnx'] = _layernorm(st['x'])
            acc_s[...] = jnp.zeros((M, D), F32)

        def mod_slice(t):
            def fn():
                st['mod'][t] = _dot(st['silu'], wm_v[:, :, _tiles(t, t + 1)].reshape(D, LANE))
            return fn

        def mod(i):
            return jnp.concatenate([st['mod'][t] for t in range(i * NS, (i + 1) * NS)], axis=1)

        def make_h():
            st['h'] = (st['lnx'] * (1.0 + mod(1)) + mod(0)).astype(BF16)

        def q_group(g):
            def fn():
                q = _dot(st['h'], wq_v[:, :, g * GD:(g + 1) * GD].reshape(D, GD))
                q_s[g] = jnp.where(diag, q, 0.0).astype(BF16)
            return fn

        def qk_slice(g, t0, t1):
            def fn():
                s = _dot(q_s[g], kbuf[g % 2, :, _tiles(t0, t1)])
                s_s[:, _tiles(t0, t1)] = s
                mx = s[:, _tiles(0, 1)]
                for u in range(1, t1 - t0):
                    mx = jnp.maximum(mx, s[:, _tiles(u, u + 1)])
                st['mx'] = mx if t0 == 0 else jnp.maximum(st['mx'], mx)
            return fn

        def row_max():
            st['m'] = jnp.max(st['mx'], axis=-1, keepdims=True)

        def pv_slice(g, t0, t1):
            def fn():
                p = jnp.exp((s_s[:, _tiles(t0, t1)] - st['m']) * scale)
                ps = p[:, _tiles(0, 1)]
                for u in range(1, t1 - t0):
                    ps = ps + p[:, _tiles(u, u + 1)]
                o = _dot_nt(p.astype(BF16), vbuf[g % 2, :, _tiles(t0, t1)])
                st['l'] = ps if t0 == 0 else st['l'] + ps
                st['o'] = o if t0 == 0 else o + st['o']
            return fn

        def normalize():
            l = jnp.sum(st['l'], axis=-1, keepdims=True)
            st['ob'] = jnp.where(diag, st['o'] / l, 0.0).astype(BF16)

        def wo_slice(t0, t1):
            def fn():
                acc_s[:, _tiles(t0, t1)] = _dot(st['ob'], wo_v[:, _tiles(t0, t1)]) + acc_s[:, _tiles(t0, t1)]
            return fn

        boxes = [(wm_hbm, wm_v, r, c, 768) for r in range(0, LANE, 8) for c in range(0, 6 * D, 768)]
        n_wm = len(boxes)
        boxes += [(wq_hbm, wq_v, r, c, 1024) for r in range(0, LANE, 8) for c in range(0, H * DH, 1024)]
        runs = ((32, 0), (64, 1), (n_wm, 0), (n_wm + 32, 2), (n_wm + 64, 0), (n_wm + 96, 1))
        head = [streams(*b, S_V + next(s for end, s in runs if i < end)) for i, b in enumerate(boxes)]
        k0_bulk = [k_piece(0, j, 0, GD - CR if j >= CARVE_K0 else GD) for j in range(NT)]
        k0_small = [[k_piece(0, j, GD - CR, CR)] if j >= CARVE_K0 else [] for j in range(NT)]
        bulk = head + k0_bulk
        wg_pieces = [rect(wg_hbm, wg_v, r, 8, c, F // 2, S_G) for r in range(0, D, 8) for c in (0, F // 2)]
        cp_c().start(priority=HI)
        cp_x().start(priority=HI)
        for i, mk in enumerate(bulk[:AHEAD]):
            mk().start(priority=LO)
            if i % (AHEAD // PRE) == AHEAD // PRE - 1:
                wg_pieces[i * PRE // AHEAD]().start(priority=HI)
        small = [[mk] for mk in wg_pieces[PRE:]] + k0_small[CARVE_K0:]
        assert len(small) == len(head) == len(bulk) - AHEAD
        work = {4: [prep]}
        for i in range(3 * NS):
            work[n_wm + 5 * i] = [mod_slice(2 * i), mod_slice(2 * i + 1)]
        work[max(work) + 1] = [make_h]
        phase([[mk] for mk in head], [[mk] for mk in bulk[AHEAD:]], small, work)

        small = wu_pieces(0) + [rect(wd_hbm, wd_v, r, 8, 0, D, S_D) for r in range(0, WD_EARLY, 8)]
        assert len(small) == CARVE0
        phase([[k0_bulk[j]] + k0_small[j] for j in range(NT)], [[v_bulk(0, j)] for j in range(NT)],
              [[mk] for mk in small] + [v_small(0, j) for j in range(CARVE0, NT)],
              {2 * g: [q_group(g)] for g in range(NG)})

        def body(g, carry):
            small = [[mk] for mk in wo_pieces(g) + wu_pieces(g + 1)]
            small += [v_small(g + 1, j) for j in range(CARVE0, NT)]
            work = {2 * i: [qk_slice(g, 4 * i, 4 * i + 4)] for i in range(8)}
            work[15] = [row_max]
            for i in range(16):
                work[16 + 2 * i] = [pv_slice(g, 2 * i, 2 * i + 2)]
            work[47] = [normalize]
            work[49] = [lambda: wait_total(wo_v, S_O), wo_slice(0, 3)]
            work[51] = [wo_slice(3, NS)]
            phase([[v_bulk(g, j)] + v_small(g, j) for j in range(NT)] + [[k_piece(g + 1, j)] for j in range(NT)],
                  [[k_piece(g + 1, j)] for j in range(NT)] + [[v_bulk(g + 1, j)] for j in range(NT)],
                  small, work)
            return carry

        lax.fori_loop(0, NG - 1, body, 0)

        g = NG - 1
        work = {j: [qk_slice(g, 3 * j, min(NT, 3 * j + 3))] for j in range(11)}
        work[11] = [row_max]
        for i in range(6):
            work[12 + i] = [pv_slice(g, 2 * i, 2 * i + 2)]
        work[20] = [lambda: wait_total(wg_v, S_G), lambda: wait_total(wu_v, S_U),
                    lambda: wait_total(wd_v.at[pl.ds(0, WD_EARLY), :], S_D)]
        for i in range(5):
            work[23 + i] = [pv_slice(g, 12 + 2 * i, 14 + 2 * i)]
        work[28] = [pv_slice(g, 22, 23)]
        work[29] = [pv_slice(g, 23, 24)]
        phase([[v_bulk(g, j)] + v_small(g, j) for j in range(NT)], [wd_last] + [[]] * (NT - 1),
              _spread(wo_pieces(g), NT - 4) + [[]] * 4, work)
        pv_slice(g, VB[2], NT)()
        normalize()

        wait_total(wo_v, S_O)
        attn = jnp.sum(_dot(st['ob'], wo_v[...]) + acc_s[...], axis=0, keepdims=True)
        x1 = st['x'] + mod(2) * attn
        h2 = (_layernorm(x1) * (1.0 + mod(4)) + mod(3)).astype(BF16)
        hh = (_dot(h2, wg_v[...]) * _dot(h2, wu_v[...])).astype(BF16)
        v0 = WD_VPU[0][0]
        hcol = jnp.broadcast_to(hh[0:1, v0:].astype(F32), (LANE, LANE)).T

        wd_last[0]().wait()
        r1 = WD_MXU[0][1]
        ffn = _dot(hh[:, :r1], wd_v[0:r1, :])
        wd_last[1]().wait()
        ffn = _dot(hh[:, r1:v0], wd_v[r1:v0, :]) + ffn
        part = None
        for mk, (a, b) in zip(wd_last[2:], WD_VPU):
            mk().wait()
            cols = [(wd_v[a:b, _tiles(t, t + 1)].astype(F32) * hcol[a - v0:b - v0])
                    .reshape((b - a) // 8, 8, LANE).sum(axis=0) for t in range(NS)]
            p8 = jnp.concatenate(cols, axis=1)
            part = p8 if part is None else part + p8
        ffn = ffn + jnp.sum(part, axis=0, keepdims=True)
        out = x1 + mod(5) * ffn
        o_ref[...] = out[0:1].reshape(1, 1, D).astype(o_ref.dtype)

    return kernel


def _compiler_params():
    vmem = 64 * 1024 * 1024
    try:
        return pltpu.CompilerParams(vmem_limit_bytes=vmem, disable_bounds_checks=True,
                                    disable_semaphore_checks=True)
    except TypeError:
        return pltpu.CompilerParams(vmem_limit_bytes=vmem)


@jax.jit
def pallas_adaLN_cond__sliding_block_cached__glu_gated_bilinear__decode_kernel(
    A_x: jax.Array,
    A_k_cache: jax.Array,
    A_v_cache: jax.Array,
    A_wq: jax.Array,
    A_wo: jax.Array,
    B_x: jax.Array,
    B_w_gate: jax.Array,
    B_w_up: jax.Array,
    B_w_down: jax.Array,
    c: jax.Array,
    w_mod: jax.Array,
):
    del B_x
    sk = A_k_cache.shape[2]
    w = min(4096, max(256, sk // 4))
    assert A_x.shape == (1, 1, D) and A_k_cache.shape == A_v_cache.shape == (1, H, sk, DH)
    assert w == NT * LANE and (sk - w) % LANE == 0
    kt = jnp.swapaxes(A_k_cache, 2, 3).reshape(H * DH, sk)
    vt = jnp.swapaxes(A_v_cache, 2, 3).reshape(H * DH, sk)
    return pl.pallas_call(
        _make_kernel(sk - w),
        out_shape=jax.ShapeDtypeStruct((1, 1, D), A_x.dtype),
        in_specs=[pl.BlockSpec(memory_space=pl.ANY)] * 10,
        scratch_shapes=[
            pltpu.VMEM((1, 1, D), BF16),
            pltpu.VMEM((1, D), BF16),
            pltpu.VMEM((NS, LANE, 6 * D), BF16),
            pltpu.VMEM((NS, LANE, H * DH), BF16),
            pltpu.VMEM((GD, D), BF16),
            pltpu.VMEM((D, F), BF16),
            pltpu.VMEM((D, F), BF16),
            pltpu.VMEM((F, D), BF16),
            pltpu.VMEM((2, GD, w), BF16),
            pltpu.VMEM((2, GD, w), BF16),
            pltpu.VMEM((NG, M, GD), BF16),
            pltpu.VMEM((M, D), F32),
            pltpu.VMEM((M, w), F32),
            pltpu.SemaphoreType.DMA((NSEM,)),
        ],
        compiler_params=_compiler_params(),
    )(A_x, c, kt, vt, A_wq.reshape(NS, LANE, H * DH), A_wo, B_w_gate, B_w_up, B_w_down,
      w_mod.reshape(NS, LANE, 6 * D))
```
